```python
import jax
import jax.numpy as jnp

def _softmax(x, axis=-1):
    return jax.nn.softmax(x, axis=axis)
def _gelu(x):
    return jax.nn.gelu(x, approximate=True)
def _silu(x):
    return jax.nn.silu(x)
def _sigmoid(x):
    return jax.nn.sigmoid(x)
def _layernorm(x, axis=-1, eps=1e-5):
    m = jnp.mean(x, axis=axis, keepdims=True)
    v = jnp.var(x, axis=axis, keepdims=True)
    return (x - m) / jnp.sqrt(v + eps)
def _scatter_add(tgt, idx, src, axis=0):
    return tgt.at[idx].add(src)
def _segment_sum(src, seg, n):
    return jax.ops.segment_sum(src, seg, n)
class _Rng:
    def __init__(self, key):
        self._k = key
    def _next(self):
        self._k, sub = jax.random.split(self._k)
        return sub
    def normal(self, shape):
        return jax.random.normal(self._next(), shape, dtype=jnp.bfloat16)
    def randint(self, lo, hi, shape):
        return jax.random.randint(self._next(), shape, lo, hi, dtype=jnp.int32)
    def uniform(self, shape, lo=0.0, hi=1.0):
        return jax.random.uniform(self._next(), shape, jnp.bfloat16, lo, hi)
    def permutation(self, n):
        return jax.random.permutation(self._next(), n)


kernel_name = 'recurrent_scan__sliding_block_cached__moe_arch_mod__decode'

def setup_inputs():
    _rng = _Rng(jax.random.key(int.from_bytes(__import__("os").urandom(4), "little")))
    _w = (lambda a: (lambda t: t.astype(jnp.bfloat16) if jnp.issubdtype(t.dtype, jnp.floating) else t)(jnp.asarray(a)))
    def _A_setup():
        B, Sq, D = 1, 1, 512
        Hq, Hkv, Sk, Dh = 32, 32, 32768, 128
        assert Hq % Hkv == 0, (Hq, Hkv)
        return {
            "x": _w((lambda *s: _rng.normal(s) * 0.05)(B, Sq, D)),
            "k_cache": _w((lambda *s: _rng.normal(s) * 0.05)(B, Hkv, Sk, Dh)),
            "v_cache": _w((lambda *s: _rng.normal(s) * 0.05)(B, Hkv, Sk, Dh)),
            "wq": _w((lambda *s: _rng.normal(s) * 0.05)(D, Hq * Dh) * (D ** -0.5)),
            "wo": _w((lambda *s: _rng.normal(s) * 0.05)(Hq * Dh, D) * ((Hq * Dh) ** -0.5)),
        }
    _A_in = _A_setup()

    def _B_setup():
        B, S, D, F, C = 1, 1, 512, 1376, 1
        return {
            "x": _w((lambda *s: _rng.normal(s) * 0.05)(B, S, D)),
            "w_r": _w((lambda *s: _rng.normal(s) * 0.05)(D)),
            "w_gate": _w((lambda *s: _rng.normal(s) * 0.05)(D, F)),
            "w_up": _w((lambda *s: _rng.normal(s) * 0.05)(D, F)),
            "w_down": _w((lambda *s: _rng.normal(s) * 0.05)(F, D)),
        }
    _B_in = _B_setup()

    return {
        "A_x": _A_in["x"],
        "A_k_cache": _A_in["k_cache"],
        "A_v_cache": _A_in["v_cache"],
        "A_wq": _A_in["wq"],
        "A_wo": _A_in["wo"],
        "B_x": _B_in["x"],
        "B_w_r": _B_in["w_r"],
        "B_w_gate": _B_in["w_gate"],
        "B_w_up": _B_in["w_up"],
        "B_w_down": _B_in["w_down"],
    }

def reference(A_x, A_k_cache, A_v_cache, A_wq, A_wo, B_x, B_w_r, B_w_gate, B_w_up, B_w_down):
    def _A_ref(x, k_cache, v_cache, wq, wo):
        B, Sq, D = x.shape
        Hq, Dh = 32, 128
        Hkv, Sk = k_cache.shape[1], k_cache.shape[2]
        W = min(4096, max(256, Sk // 4))
        rep = Hq // Hkv
        q = (lambda x, *d: x.transpose(*d))((x @ wq).reshape(B, Sq, Hq, Dh), 0, 2, 1, 3)
        k = jnp.repeat(k_cache[:, :, Sk - W:, :], rep, axis=1)
        v = jnp.repeat(v_cache[:, :, Sk - W:, :], rep, axis=1)
        scores = jnp.einsum("bhqd,bhkd->bhqk", q, k) * (Dh ** -0.5)
        p = _softmax(scores, axis=-1)
        o = jnp.einsum("bhqk,bhkd->bhqd", p, v)
        return (lambda x, *d: x.transpose(*d))(o, 0, 2, 1, 3).reshape(B, Sq, Hq * Dh) @ wo

    def _B_ref(x, w_r, w_gate, w_up, w_down):
        B, S, D = x.shape
        C = 1
        r = x @ w_r
        idx = jnp.argsort(-r, axis=-1)[:, :C]
        idx_e = jnp.repeat(idx.reshape(B, C, 1), D, axis=2)
        x_sel = jnp.take_along_axis(x, idx_e, axis=1)
        g = _silu(x_sel @ w_gate)
        u = x_sel @ w_up
        y = (g * u) @ w_down
        r_sel = _sigmoid(jnp.take_along_axis(r, idx, axis=1))
        y = y * r_sel.reshape(B, C, 1)
        b_off = (jnp.arange(B) * S).reshape(B, 1)
        flat_idx = (idx + b_off).reshape(B * C)
        zero = (x * 0.0).reshape(B * S, D)
        upd = _scatter_add(zero, flat_idx, y.reshape(B * C, D), axis=0)
        return x + upd.reshape(B, S, D)

    x = A_x
    xn = _layernorm(x, axis=-1)
    s = _A_ref(xn, A_k_cache, A_v_cache, A_wq, A_wo)
    g = _silu(_B_ref(xn, B_w_r, B_w_gate, B_w_up, B_w_down))
    return x + s * g
```

```python
import jax
import jax.numpy as jnp
import jax.experimental.pallas as pl
import jax.experimental.pallas.tpu as pltpu

D, NH, DH, SK, F = 512, 32, 128, 32768, 1376
W = min(4096, max(256, SK // 4))
BF16, F32 = jnp.bfloat16, jnp.float32
_NT = (((1,), (1,)), ((), ()))
LONG, SHORT = 1, 0

DEF = dict(K0=128, V0=64, O0=32, t_idle=120, t_q=0, t_qk=58, t_sm=0, t_gu=58, t_pv=58, t_y=0, t_o=0, t_end=118,
           s_pv=646, y2=True, o2=True, t_o2=40, manual_out=False, nowait=False,
           wo=((0, 8, 32, 64, 0), (0, 8, 96, 64, 0), (0, 8, 160, 64, 0), (0, 8, 224, 64, 0), (0, 4, 288, 64, 1), (0, 4, 352, 64, 1),
               (0, 4, 416, 64, 2), (4, 4, 288, 64, 3), (4, 4, 352, 64, 3), (4, 2, 416, 64, 4), (6, 1, 416, 64, 5),
               (7, 1, 416, 32, 6), (7, 1, 448, 16, 7), (7, 1, 464, 16, 8)),
           end='c6,7 i786 w0 a1 E a0 w1 s h2,0,1,2,3 s60 w2 e0,1,2,3 s h3,0,1,2,3 s70 s80 s80 s80 s w3 h2,4,5,6,7 v6,384,32 v7,384,32 '
               'w4 e4,5 h3,4,5 w5 e6 v6,416,96 e7 v7,480,32 w6 v7,416,32 w7 v7,448,16 w8 v7,464,16')


def make(name=None, **kw):
    P = dict(DEF); P.update(kw)
    K0, V0, O0 = P['K0'], P['V0'], P['O0']
    BR, PR = 256, 64
    NB = W // BR - 1
    NS, SR, OB, OP = 8, 512, 64, 16
    NOB = SR // OB - 1
    NF = F // OP
    S_KE = 256; S_G = S_KE + 128; S_U = S_G + NF; S_VE = S_U + NF; S_D = S_VE + 128; S_O = S_D + NF; S_END = S_O + 32
    NL = 2 * NB
    UE = 8

    def kernel(x_h, k_h, v_h, wq_h, wo_h, wr_h, wg_h, wu_h, wd_h, out_ref,
               x_v, wr_v, wq_v, k_v, v_v, wo_v, wg_v, wu_v, wd_v, q_v, s_v, o_v, h_v, res_v,
               s_x, s_p, s_l, s_o1, s_o0):
        def wait(c):
            if not P['nowait']: c.wait()

        def long_kv(t, b, n):
            src, dst, r0 = ((k_h, k_v, K0), (v_h, v_v, V0))[t]
            r = r0 + b * BR
            if not isinstance(r, int): r = pl.multiple_of(r, PR)
            return pltpu.make_async_copy(src.at[0, :, pl.ds(SK - W + r, BR), :], dst.at[:, pl.ds(r - V0, BR), :], s_l.at[n])

        def long_wo(s0, ns, r, nr, i):
            return pltpu.make_async_copy(wo_h.at[pl.ds(s0, ns), pl.ds(r, nr), :], wo_v.at[pl.ds(s0, ns), pl.ds(r, nr), :], s_o1.at[i])

        wo_long = [long_wo(s0, ns, r, nr, i) for s0, ns, r, nr, i in P['wo']]

        def piece_wq(i):
            r, c = pl.multiple_of((i >> 2) * 8, 8), pl.multiple_of((i & 3) * 1024, 1024)
            return pltpu.make_async_copy(wq_h.at[pl.ds(r, 8), pl.ds(c, 1024)], wq_v.at[pl.ds(r, 8), pl.ds(c, 1024)], s_p.at[0])

        def piece_kv(src, dst, r0, sem):
            def f(i):
                r = (r0 + NB * BR + (i & 3) * PR) & (W - 1)
                return pltpu.make_async_copy(src.at[0, i >> 2, pl.ds(pl.multiple_of(SK - W + r, PR), PR), :],
                                             dst.at[i >> 2, pl.ds(pl.multiple_of((r - V0) & (W - 1), PR), PR), :], sem)
            return f

        def piece_w(src, dst, sem):
            def f(i):
                r = pl.multiple_of(i * OP, OP)
                return pltpu.make_async_copy(src.at[pl.ds(r, OP), :], dst.at[pl.ds(r, OP), :], s_p.at[sem])
            return f

        def piece_wo(i):
            s = (i >> 1) & (NS - 1)
            r = (i >> 4) * (SR - 2 * OP) + (i & 1) * OP
            sem = (i >> 4) * (1 + s)
            if not isinstance(r, int): r = pl.multiple_of(r, OP)
            return pltpu.make_async_copy(wo_h.at[s, pl.ds(r, OP), :], wo_v.at[s, pl.ds(r, OP), :], s_o0.at[sem])

        cargo = ((0, S_KE, piece_wq), (S_KE, S_G, piece_kv(k_h, k_v, K0, s_l.at[1])), (S_G, S_U, piece_w(wg_h, wg_v, 2)),
                 (S_U, S_VE, piece_w(wu_h, wu_v, 3)), (S_VE, S_D, piece_kv(v_h, v_v, V0, s_l.at[2 + UE])),
                 (S_D, S_O, piece_w(wd_h, wd_v, 5)), (S_O, S_END, piece_wo))

        def wait_all(ref, sem):
            wait(pltpu.make_async_copy(ref, ref, sem))

        def issue(s, lo, hi):
            kinds = [c for c in cargo if c[0] < hi and c[1] > lo]
            for a, b, f in kinds:
                if len(kinds) == 1:
                    f(s - a).start(priority=SHORT)
                else:
                    pl.when((s >= a) & (s < b))(lambda: f(s - a).start(priority=SHORT))

        pos = [0]

        def run(n, t, work=None, carry=0, two=False):
            lo = pos[0]; hi = pos[0] = lo + n * (1 + two)

            def body(i, c):
                s = lo + i * (1 + two)
                issue(s, lo, hi)
                if two:
                    pl.delay(t)
                    issue(s + 1, lo, hi)
                if work is not None: c = work(i, c)
                if t and not two: pl.delay(t)
                return c
            if P.get('scopes'):
                with jax.named_scope(f'sc_{lo:03d}_{hi - lo}'): return jax.lax.fori_loop(0, n, body, carry)
            return jax.lax.fori_loop(0, n, body, carry)

        def idle_until(s):
            assert s >= pos[0], (s, pos[0])
            if s > pos[0]: run(s - pos[0], P['t_idle'])

        long_kv(0, 0, 0).start(priority=LONG)
        copy_x = pltpu.make_async_copy(x_h, x_v, s_x.at[0])
        copy_wr = pltpu.make_async_copy(wr_h, wr_v, s_x.at[1])
        copy_x.start(priority=SHORT)
        copy_wr.start(priority=SHORT)
        KS = 10

        @pl.loop(1, NB)
        def _(b):
            long_kv(0, b, (b >= KS).astype(jnp.int32)).start(priority=LONG)

        row = jax.lax.broadcasted_iota(jnp.int32, (8, DH), 0)
        q_v[...] = jnp.zeros(q_v.shape, F32)
        o_v[...] = jnp.zeros(o_v.shape, F32)

        idle_until(S_KE)

        @pl.loop(0, NB)
        def _(b):
            long_kv(1, b, 2 + b + (b >= UE).astype(jnp.int32)).start(priority=LONG)
        idle_until(S_KE + 5)
        copy_x.wait()
        copy_wr.wait()
        x = x_v[0].astype(F32)
        mean = jnp.mean(x, axis=-1, keepdims=True)
        var = jnp.mean(jnp.square(x - mean), axis=-1, keepdims=True)
        xn_b = ((x - mean) / jnp.sqrt(var + 1e-5)).astype(BF16)
        xn = xn_b.astype(F32)
        xn8 = jnp.broadcast_to(xn_b, (8, D))

        wait_all(wq_v, s_p.at[0])

        def q_proj(h, c):
            q = jnp.dot(xn8, wq_v[:, pl.ds(pl.multiple_of(h * DH, DH), DH)], preferred_element_type=F32)
            q_v[h >> 3] = jnp.where(row == (h & 7), q, q_v[h >> 3])
            return c
        run(NH, P['t_q'], q_proj)

        def per_head(g, f):
            r = f(g * 8)
            for j in range(1, 8):
                r = jnp.where(row == j, f(g * 8 + j), r)
            return r

        IE = 64
        assert pos[0] + 2 * IE >= S_G + 5
        assert (128 * ((IE - 1) // 4 + 1) + 127) // 256 < KS
        wait_all(k_v.at[:, pl.ds(0, KS * BR), :], s_l.at[0])

        def qk(i, c):
            g, t = i & 3, ((i >> 2) + 1) & 31
            pl.when(i == IE)(lambda: wait_all(k_v.at[:, pl.ds(KS * BR, W - KS * BR), :], s_l.at[1]))
            q = q_v[g].astype(BF16)
            rows = pl.ds(pl.multiple_of(t * DH, DH), DH)
            s_v[g, t] = per_head(g, lambda h: jax.lax.dot_general(q, k_v[h, rows, :], _NT, preferred_element_type=F32)) * (DH ** -0.5)
            return c
        run(NH // 8 * (W // DH), P['t_qk'], qk, two=True)

        def softmax(g, c):
            s = s_v[g]
            p = jnp.exp(s - jnp.max(jnp.max(s, axis=0), axis=-1, keepdims=True))
            s_v[g] = p
            q_v[g] = jnp.sum(p, axis=0)
            return c
        run(NH // 8, P['t_sm'], softmax)

        idle_until(max(pos[0], S_VE + 5))
        wait_all(wg_v, s_p.at[2])
        wait_all(wu_v, s_p.at[3])
        NC = -(-F // DH)
        lane = jax.lax.broadcasted_iota(jnp.int32, (8, DH), 1)
        chunk = lambda i: pl.ds(pl.multiple_of(jnp.minimum(i * DH, F - DH), 32), DH)

        def gate_up(i, c):
            gt = jax.lax.dot_general(xn8, wg_v[chunk(i), :], _NT, preferred_element_type=F32)
            up = jax.lax.dot_general(xn8, wu_v[chunk(i), :], _NT, preferred_element_type=F32)
            h_v[i] = jnp.where(lane >= (i + 1) * DH - F, jax.nn.silu(gt) * up, 0.0)
            return c
        run(NC, P['t_gu'], gate_up, two=True)
        r = jnp.sum(xn * wr_v[...].reshape(1, D).astype(F32), axis=-1, keepdims=True)

        idle_until(P['s_pv'])
        for c in wo_long:
            c.start(priority=LONG)
            pl.delay(1)

        def pv2(i, c):
            u = i >> 2
            pl.when(i & 3 == 0)(lambda: wait_all(v_v.at[:, pl.ds(0, BR), :], s_l.at[2 + u]))
            u = jnp.where(u == UE, NB, u - (u > UE).astype(jnp.int32))
            g = i & 3
            p = jnp.concatenate([s_v[g, 2 * u], s_v[g, 2 * u + 1]], axis=1).astype(BF16)
            rows = pl.ds(pl.multiple_of(u * BR, BR), BR)
            o_v[g] += per_head(g, lambda h: jnp.dot(p, v_v[h, rows, :], preferred_element_type=F32))
            return c
        run(NH // 8 * (W // BR), P['t_pv'], pv2, two=True)
        for g in range(NH // 8):
            o_v[g] = o_v[g] / jnp.sum(q_v[g], axis=-1, keepdims=True)

        idle_until(max(pos[0], S_O + 4))
        wait_all(wd_v, s_p.at[5])
        down = lambda i: jnp.dot(h_v[i].astype(BF16), wd_v[chunk(i), :], preferred_element_type=F32)
        if P.get('y2'): y = run(NC // 2, 0, lambda i, y: y + down(2 * i) + down(2 * i + 1), down(NC - 1))
        else: y = run(NC, P['t_y'], lambda i, y: y + down(i), jnp.zeros((8, D), F32))
        gate = jax.nn.silu(xn + (xn * 0.0 + y * jax.nn.sigmoid(r)))
        row_d = jax.lax.broadcasted_iota(jnp.int32, (8, D), 0)

        def head(acc, s, a):
            r = a * DH
            if not isinstance(r, int): r = pl.multiple_of(r, DH)
            t = jnp.dot(o_v[s >> 1].astype(BF16), wo_v[s, pl.ds(r, DH), :], preferred_element_type=F32)
            return acc + jnp.where(row_d == (s & 1) * 4 + a, t, 0.0)

        def o_proj(a):
            return lambda g, acc: head(head(acc, 2 * g, a), 2 * g + 1, a)

        cols = {}

        def vpu(acc, s, r, nr):
            coef = jnp.concatenate([cols[s][r - 3 * DH:r - 3 * DH + nr]] * (D // DH), axis=1)
            return acc + (wo_v[s, pl.ds(r, nr), :].astype(F32) * coef).reshape(nr // 8, 8, D).sum(axis=0)

        acc = jnp.zeros((8, D), F32)
        for n, it in enumerate(P['end'].split()):
            k, v = it[0], [int(z) for z in it[1:].split(',') if z]
            if k == 'i': idle_until(v[0])
            elif k == 'a': acc = run(4, 0, o_proj(v[0]), acc)
            elif k == 's':
                pl.delay(1)
                piece_wo(pos[0] - S_O).start(priority=SHORT)
                pl.delay(v[0] if v else 1)
                pos[0] += 1
            elif k == 'w':
                for c, d in zip(wo_long, P['wo']):
                    if d[4] == v[0]: wait(c)
            elif k == 'E': wait_all(wo_v.at[:, pl.ds(0, 2 * OP), :], s_o0.at[0])
            elif k == 'e':
                for z in v: wait_all(wo_v.at[z, pl.ds(0, 2 * OP), :], s_o0.at[1 + z])
            elif k == 'h':
                for z in v[1:]: acc = head(acc, z, v[0])
            elif k == 'c':
                for z in v:
                    j = (z & 1) * 4 + 3
                    cols[z] = jnp.broadcast_to(o_v[z >> 1].astype(BF16).astype(F32)[j:j + 1], (DH, DH)).T
            elif k == 'v': acc = vpu(acc, *v)
            if k in 'weE' and P.get('scopes'):
                with jax.named_scope(f'sc_9{n:02d}{it}_1'): pl.delay(1)
        assert pos[0] == S_END, pos[0]
        res = jnp.broadcast_to(x, (8, D)) + jnp.broadcast_to(jnp.sum(acc, axis=0, keepdims=True), (8, D)) * gate
        if P['manual_out']:
            res_v[0] = res.astype(BF16)[0:1]
            c = pltpu.make_async_copy(res_v, out_ref, s_x.at[0]); c.start(); c.wait()
        else:
            out_ref[0] = res.astype(BF16)[0:1]

    def fn(A_x, A_k_cache, A_v_cache, A_wq, A_wo, B_x, B_w_r, B_w_gate, B_w_up, B_w_down):
        hbm = pl.BlockSpec(memory_space=pltpu.HBM)
        dma = pltpu.SemaphoreType.DMA
        return pl.pallas_call(
            kernel, name=name,
            out_shape=jax.ShapeDtypeStruct((1, 1, D), BF16),
            in_specs=[hbm] * 9,
            out_specs=hbm if P['manual_out'] else pl.BlockSpec(memory_space=pltpu.VMEM),
            scratch_shapes=[
                pltpu.VMEM((1, 1, D), BF16), pltpu.VMEM((D,), BF16), pltpu.VMEM((D, NH * DH), BF16),
                pltpu.VMEM((NH, W, DH), BF16), pltpu.VMEM((NH, W, DH), BF16), pltpu.VMEM((NS, SR, D), BF16),
                pltpu.VMEM((F, D), BF16), pltpu.VMEM((F, D), BF16), pltpu.VMEM((F, D), BF16),
                pltpu.VMEM((NH // 8, 8, DH), F32), pltpu.VMEM((NH // 8, W // DH, 8, DH), F32), pltpu.VMEM((NH // 8, 8, DH), F32),
                pltpu.VMEM((-(-F // DH), 8, DH), F32), pltpu.VMEM((1, 1, D), BF16),
                dma((2,)), dma((6,)), dma((3 + NB,)), dma((P['wo'][-1][4] + 1,)), dma((1 + NS,)),
            ],
            compiler_params=pltpu.CompilerParams(vmem_limit_bytes=100 * 1024 * 1024, disable_semaphore_checks=True,
                                                 disable_bounds_checks=True),
        )(A_x, A_k_cache, A_v_cache, A_wq, A_wo.reshape(NS, SR, D), B_w_r, B_w_gate.T, B_w_up.T, B_w_down)
    return fn


pallas_recurrent_scan__sliding_block_cached__moe_arch_mod__decode_kernel = jax.jit(make())
```

```python
import jax
import jax.numpy as jnp
import jax.experimental.pallas as pl
import jax.experimental.pallas.tpu as pltpu

D, NH, DH, SK, F = 512, 32, 128, 32768, 1376
W = min(4096, max(256, SK // 4))
BF16, F32 = jnp.bfloat16, jnp.float32
_NT = (((1,), (1,)), ((), ()))
LONG, SHORT = 1, 0

DEF = dict(K0=128, V0=64, O0=32, t_idle=114, t_q=0, t_qk=51, t_sm=0, t_gu=54, t_pv=50, t_y=0, t_o=0, t_end=118,
           s_pv=676, y2=True, o2=True, t_o2=40, manual_out=False, nowait=False,
           ue=13, last=(32, 16, 16), t_n=20, t_c=20, t_a0=0, unroll=False)


def make(name=None, **kw):
    P = dict(DEF); P.update(kw)
    K0, V0, O0 = P['K0'], P['V0'], P['O0']
    BR, PR = 256, 64
    NB = W // BR - 1
    NS, SR, OB, OP = 8, 512, 64, 16
    NOB = SR // OB - 1
    NF = F // OP
    S_KE = 256; S_G = S_KE + 128; S_U = S_G + NF; S_D = S_U + NF; S_VE = S_D + NF; S_O = S_VE + 128; S_L = S_O + 32; S_END = S_L + 28
    NL = 2 * NB
    UE = P['ue']

    def kernel(x_h, k_h, v_h, wq_h, wo_h, wr_h, wg_h, wu_h, wd_h, out_ref,
               x_v, wr_v, wq_v, k_v, v_v, wo_v, wg_v, wu_v, wd_v, q_v, s_v, o_v, h_v, res_v, c_v,
               s_x, s_p, s_l, s_o1):
        def wait(c):
            if not P['nowait']: c.wait()

        def long_kv(t, b, n):
            src, dst, r0 = ((k_h, k_v, K0), (v_h, v_v, V0))[t]
            r = r0 + b * BR
            if not isinstance(r, int): r = pl.multiple_of(r, PR)
            return pltpu.make_async_copy(src.at[0, :, pl.ds(SK - W + r, BR), :], dst.at[:, pl.ds(r - V0, BR), :], s_l.at[n])

        def long_wo(s0, ns, r, nr, i):
            return pltpu.make_async_copy(wo_h.at[pl.ds(s0, ns), pl.ds(r, nr), :], wo_v.at[pl.ds(s0, ns), pl.ds(r, nr), :], s_o1.at[i])

        RL = O0 + (NOB - 1) * OB

        def wo_block(q):
            j = jnp.where(q == 0, 5, jnp.where(q == 6, 6, q - 1))
            return O0 + j * OB, jnp.where(q == 6, 3 + NS - 1, jnp.maximum((q - 1) >> 1, 0))

        def piece_wq(i):
            r, c = pl.multiple_of((i >> 2) * 8, 8), pl.multiple_of((i & 3) * 1024, 1024)
            return pltpu.make_async_copy(wq_h.at[pl.ds(r, 8), pl.ds(c, 1024)], wq_v.at[pl.ds(r, 8), pl.ds(c, 1024)], s_p.at[0])

        def piece_kv(src, dst, r0, sem):
            def f(i):
                r = (r0 + NB * BR + (i & 3) * PR) & (W - 1)
                return pltpu.make_async_copy(src.at[0, i >> 2, pl.ds(pl.multiple_of(SK - W + r, PR), PR), :],
                                             dst.at[i >> 2, pl.ds(pl.multiple_of((r - V0) & (W - 1), PR), PR), :], sem)
            return f

        def piece_w(src, dst, sem):
            def f(i):
                r = pl.multiple_of(i * OP, OP)
                return pltpu.make_async_copy(src.at[pl.ds(r, OP), :], dst.at[pl.ds(r, OP), :], s_p.at[sem])
            return f

        def piece_wo(i):
            r = pl.multiple_of((O0 + NOB * OB + (i & 3) * OP) & (SR - 1), OP)
            return pltpu.make_async_copy(wo_h.at[i >> 2, pl.ds(r, OP), :], wo_v.at[i >> 2, pl.ds(r, OP), :], s_o1.at[0])

        def piece_last(i):
            r, sem = wo_block(i >> 2)
            r = pl.multiple_of(r + (i & 3) * OP, OP)
            return pltpu.make_async_copy(wo_h.at[NS - 1, pl.ds(r, OP), :], wo_v.at[NS - 1, pl.ds(r, OP), :], s_o1.at[sem])

        cargo = ((0, S_KE, piece_wq), (S_KE, S_G, piece_kv(k_h, k_v, K0, s_l.at[1])), (S_G, S_U, piece_w(wg_h, wg_v, 2)),
                 (S_U, S_D, piece_w(wu_h, wu_v, 3)), (S_D, S_VE, piece_w(wd_h, wd_v, 5)),
                 (S_VE, S_O, piece_kv(v_h, v_v, V0, s_l.at[2 + UE])), (S_O, S_L, piece_wo), (S_L, S_END, piece_last))

        def wait_all(ref, sem):
            wait(pltpu.make_async_copy(ref, ref, sem))

        def issue(s, lo, hi):
            kinds = [c for c in cargo if c[0] < hi and c[1] > lo]
            for a, b, f in kinds:
                if len(kinds) == 1:
                    f(s - a).start(priority=SHORT)
                else:
                    pl.when((s >= a) & (s < b))(lambda: f(s - a).start(priority=SHORT))

        pos = [0]

        def run(n, t, work=None, carry=0, two=False):
            lo = pos[0]; hi = pos[0] = lo + n * (1 + two)

            def body(i, c):
                s = lo + i * (1 + two)
                issue(s, lo, hi)
                if two:
                    pl.delay(t)
                    issue(s + 1, lo, hi)
                if work is not None: c = work(i, c)
                if t and not two: pl.delay(t)
                return c
            if P.get('scopes'):
                with jax.named_scope(f'sc_{lo:03d}_{hi - lo}'): return jax.lax.fori_loop(0, n, body, carry)
            return jax.lax.fori_loop(0, n, body, carry)

        def idle_until(s):
            assert s >= pos[0], (s, pos[0])
            if s > pos[0]: run(s - pos[0], P['t_idle'])

        long_kv(0, 0, 0).start(priority=LONG)
        copy_x = pltpu.make_async_copy(x_h, x_v, s_x.at[0])
        copy_wr = pltpu.make_async_copy(wr_h, wr_v, s_x.at[1])
        copy_x.start(priority=SHORT)
        copy_wr.start(priority=SHORT)
        KS = 10

        @pl.loop(1, NB)
        def _(b):
            long_kv(0, b, (b >= KS).astype(jnp.int32)).start(priority=LONG)

        row = jax.lax.broadcasted_iota(jnp.int32, (8, DH), 0)
        q_v[...] = jnp.zeros(q_v.shape, F32)
        o_v[...] = jnp.zeros(o_v.shape, F32)

        idle_until(S_KE)

        @pl.loop(0, NB)
        def _(b):
            long_kv(1, b, 2 + b + (b >= UE).astype(jnp.int32)).start(priority=LONG)
        idle_until(S_KE + 5)
        copy_x.wait()
        copy_wr.wait()
        x = x_v[0].astype(F32)
        mean = jnp.mean(x, axis=-1, keepdims=True)
        var = jnp.mean(jnp.square(x - mean), axis=-1, keepdims=True)
        xn_b = ((x - mean) / jnp.sqrt(var + 1e-5)).astype(BF16)
        xn = xn_b.astype(F32)
        xn8 = jnp.broadcast_to(xn_b, (8, D))

        wait_all(wq_v, s_p.at[0])

        def q_proj(h, c):
            q = jnp.dot(xn8, wq_v[:, pl.ds(pl.multiple_of(h * DH, DH), DH)], preferred_element_type=F32)
            q_v[h >> 3] = jnp.where(row == (h & 7), q, q_v[h >> 3])
            return c
        run(NH, P['t_q'], q_proj)

        def per_head(g, f):
            r = f(g * 8)
            for j in range(1, 8):
                r = jnp.where(row == j, f(g * 8 + j), r)
            return r

        IE = 64
        assert pos[0] + 2 * IE >= S_G + 5
        assert (128 * ((IE - 1) // 4 + 1) + 127) // 256 < KS
        wait_all(k_v.at[:, pl.ds(0, KS * BR), :], s_l.at[0])

        def qk(i, c):
            g, t = i & 3, ((i >> 2) + 1) & 31
            pl.when(i == IE)(lambda: wait_all(k_v.at[:, pl.ds(KS * BR, W - KS * BR), :], s_l.at[1]))
            q = q_v[g].astype(BF16)
            rows = pl.ds(pl.multiple_of(t * DH, DH), DH)
            s_v[g, t] = per_head(g, lambda h: jax.lax.dot_general(q, k_v[h, rows, :], _NT, preferred_element_type=F32)) * (DH ** -0.5)
            return c
        run(NH // 8 * (W // DH), P['t_qk'], qk, two=True)

        def softmax(g, c):
            s = s_v[g]
            p = jnp.exp(s - jnp.max(jnp.max(s, axis=0), axis=-1, keepdims=True))
            s_v[g] = p
            q_v[g] = jnp.sum(p, axis=0)
            return c
        run(NH // 8, P['t_sm'], softmax)

        idle_until(max(pos[0], S_D + 5))
        wait_all(wg_v, s_p.at[2])
        wait_all(wu_v, s_p.at[3])
        NC = -(-F // DH)
        lane = jax.lax.broadcasted_iota(jnp.int32, (8, DH), 1)
        chunk = lambda i: pl.ds(pl.multiple_of(jnp.minimum(i * DH, F - DH), 32), DH)

        def gate_up(i, c):
            gt = jax.lax.dot_general(xn8, wg_v[chunk(i), :], _NT, preferred_element_type=F32)
            up = jax.lax.dot_general(xn8, wu_v[chunk(i), :], _NT, preferred_element_type=F32)
            h_v[i] = jnp.where(lane >= (i + 1) * DH - F, jax.nn.silu(gt) * up, 0.0)
            return c
        run(NC, P['t_gu'], gate_up, two=True)
        r = jnp.sum(xn * wr_v[...].reshape(1, D).astype(F32), axis=-1, keepdims=True)

        idle_until(max(pos[0], S_VE + 5))
        wait_all(wd_v, s_p.at[5])
        down = lambda i: jnp.dot(h_v[i].astype(BF16), wd_v[chunk(i), :], preferred_element_type=F32)
        if P.get('y2'): y = run(NC // 2, 0, lambda i, y: y + down(2 * i) + down(2 * i + 1), down(NC - 1))
        else: y = run(NC, P['t_y'], lambda i, y: y + down(i), jnp.zeros((8, D), F32))
        gate = jax.nn.silu(xn + (xn * 0.0 + y * jax.nn.sigmoid(r)))
        idle_until(P['s_pv'])
        assert pos[0] + 8 * UE >= S_O + 4

        @pl.loop(0, NOB - 1)
        def _(q):
            r, sem = wo_block(q)
            long_wo(0, NS - 1, pl.multiple_of(r, OP), OB, sem).start(priority=LONG)

        @pl.loop(0, NS - 2)
        def _(z):
            long_wo(z, 1, RL, OB, 3 + z).start(priority=LONG)
        last = []; r = RL
        for i, nr in enumerate(P['last']):
            last.append((long_wo(NS - 2, 1, r, nr, 3 + NS - 2 if i == 0 else 2 + NS + i), r, nr)); r += nr
            last[-1][0].start(priority=LONG)

        def pv2(i, c):
            u = i >> 2
            pl.when(i & 3 == 0)(lambda: wait_all(v_v.at[:, pl.ds(0, BR), :], s_l.at[2 + u]))
            u = jnp.where(u == UE, NB, u - (u > UE).astype(jnp.int32))
            g = i & 3
            p = jnp.concatenate([s_v[g, 2 * u], s_v[g, 2 * u + 1]], axis=1).astype(BF16)
            rows = pl.ds(pl.multiple_of(u * BR, BR), BR)
            o_v[g] += per_head(g, lambda h: jnp.dot(p, v_v[h, rows, :], preferred_element_type=F32))
            return c
        run(NH // 8 * (W // BR), P['t_pv'], pv2, two=True)

        def normalize(g, c):
            o_v[g] = o_v[g] / jnp.sum(q_v[g], axis=-1, keepdims=True)
            return c
        run(NH // 8, P['t_n'], normalize)

        def columns(g, c):
            o = o_v[g].astype(BF16).astype(F32)
            for z in range(2):
                c_v[2 * g + z] = jnp.broadcast_to(o[4 * z + 3:4 * z + 4], (DH, DH)).T
            return c
        run(NH // 8, P['t_c'], columns, two=True)
        row_d = jax.lax.broadcasted_iota(jnp.int32, (8, D), 0)

        def head(acc, s, a):
            r = a * DH
            if not isinstance(r, int): r = pl.multiple_of(r, DH)
            t = jnp.dot(o_v[s >> 1].astype(BF16), wo_v[s, pl.ds(r, DH), :], preferred_element_type=F32)
            return acc + jnp.where(row_d == (s & 1) * 4 + a, t, 0.0)

        def o_proj(a):
            return lambda g, acc: head(head(acc, 2 * g, a), 2 * g + 1, a)

        def vpu(acc, z, r, nr):
            coef = jnp.concatenate([c_v[z, pl.ds(r - 3 * DH, nr), :]] * (D // DH), axis=1)
            return acc + (wo_v[z, pl.ds(r, nr), :].astype(F32) * coef).reshape(nr // 8, 8, D).sum(axis=0)

        def mark(n):
            if P.get('scopes'):
                with jax.named_scope(f'sc_9{n}_1'): pl.delay(1)

        idle_until(S_END - 12)
        wait_all(wo_v.at[:, pl.ds(0, 4 * OB), :], s_o1.at[0])
        acc = run(NS, P['t_a0'], lambda z, acc: head(vpu(vpu(acc, z, 3 * DH, RL - 3 * DH), z, RL + OB, SR - RL - OB), z, 0),
                  jnp.zeros((8, D), F32))
        wait_all(wo_v.at[:, pl.ds(0, 2 * OB), :], s_o1.at[1])
        acc = run(4, 0, o_proj(1), acc)
        mark(0)
        wait_all(wo_v.at[:, pl.ds(0, OB), :], s_o1.at[2])
        mark(1)
        for z in range(NS): acc = head(acc, z, 2)
        mark(2)

        def tail(z, acc):
            long_wo(z, 1, RL, OB, 3 + z).wait()
            return vpu(acc, z, RL, OB)
        acc = jax.lax.fori_loop(0, NS - 2, tail, acc, unroll=P['unroll'])
        mark(3)
        acc = tail(NS - 1, acc)
        mark(4)
        for c, r, nr in last:
            c.wait()
            acc = vpu(acc, NS - 2, r, nr)
        res = jnp.broadcast_to(x, (8, D)) + jnp.broadcast_to(jnp.sum(acc, axis=0, keepdims=True), (8, D)) * gate
        if P['manual_out']:
            res_v[0] = res.astype(BF16)[0:1]
            c = pltpu.make_async_copy(res_v, out_ref, s_x.at[0]); c.start(); c.wait()
        else:
            out_ref[0] = res.astype(BF16)[0:1]

    def fn(A_x, A_k_cache, A_v_cache, A_wq, A_wo, B_x, B_w_r, B_w_gate, B_w_up, B_w_down):
        hbm = pl.BlockSpec(memory_space=pltpu.HBM)
        dma = pltpu.SemaphoreType.DMA
        return pl.pallas_call(
            kernel, name=name,
            out_shape=jax.ShapeDtypeStruct((1, 1, D), BF16),
            in_specs=[hbm] * 9,
            out_specs=hbm if P['manual_out'] else pl.BlockSpec(memory_space=pltpu.VMEM),
            scratch_shapes=[
                pltpu.VMEM((1, 1, D), BF16), pltpu.VMEM((D,), BF16), pltpu.VMEM((D, NH * DH), BF16),
                pltpu.VMEM((NH, W, DH), BF16), pltpu.VMEM((NH, W, DH), BF16), pltpu.VMEM((NS, SR, D), BF16),
                pltpu.VMEM((F, D), BF16), pltpu.VMEM((F, D), BF16), pltpu.VMEM((F, D), BF16),
                pltpu.VMEM((NH // 8, 8, DH), F32), pltpu.VMEM((NH // 8, W // DH, 8, DH), F32), pltpu.VMEM((NH // 8, 8, DH), F32),
                pltpu.VMEM((-(-F // DH), 8, DH), F32), pltpu.VMEM((1, 1, D), BF16), pltpu.VMEM((NS, DH, DH), F32),
                dma((2,)), dma((6,)), dma((3 + NB,)), dma((2 + NS + len(P['last']),)),
            ],
            compiler_params=pltpu.CompilerParams(vmem_limit_bytes=100 * 1024 * 1024, disable_semaphore_checks=True,
                                                 disable_bounds_checks=True),
        )(A_x, A_k_cache, A_v_cache, A_wq, A_wo.reshape(NS, SR, D), B_w_r, B_w_gate.T, B_w_up.T, B_w_down)
    return fn


pallas_recurrent_scan__sliding_block_cached__moe_arch_mod__decode_kernel = jax.jit(make())
```

```python
import jax
import jax.numpy as jnp
import jax.experimental.pallas as pl
import jax.experimental.pallas.tpu as pltpu

D = 512
NH = 32
DH = 128
SK = 32768
W = min(4096, max(256, SK // 4))
F = 1376
NG = NH // 8
NT = W // DH
NC = -(-F // DH)

BR, PR = 256, 32
NB = W // BR - 1
K0, V0 = 128, 64
NS, SR = 8, 512
OB, OP = 64, 8
NOB = SR // OB - 1
O0 = 32
RL = O0 + (NOB - 1) * OB
LAST = (32, 16, 16)

S_K = D * NH * DH // (OP * D)
S_G = S_K + NH * BR // PR
S_U = S_G + F // OP
S_D = S_U + F // OP
S_V = S_D + F // OP
S_O = S_V + NH * BR // PR
S_L = S_O + NS * OB // OP
S_END = S_L + NOB * OB // OP
LAND = 12
S_PV = 1356
KB, KI = 10, 64
VE = 13
BURST, T_BURST = 16, 14
T_IDLE, T_Q, T_QK, T_FFN, T_PV, T_O = 59, 24, 17, 20, 15, 14

BF16 = jnp.bfloat16
F32 = jnp.float32
_NT = (((1,), (1,)), ((), ()))
LONG, SHORT = 1, 0


def _rows(start, size, multiple):
    return pl.ds(start if isinstance(start, int) else pl.multiple_of(start, multiple), size)


def _kernel(x_h, k_h, v_h, wq_h, wo_h, wr_h, wg_h, wu_h, wd_h, out_ref,
            x_v, wr_v, wq_v, k_v, v_v, wo_v, wg_v, wu_v, wd_v, q_v, s_v, l_v, o_v, h_v, c_v,
            sem_x, sem_w, sem_k, sem_v, sem_o):
    def long_kv(src, dst, r0, b, sem):
        r = r0 + b * BR
        return pltpu.make_async_copy(src.at[0, :, _rows(SK - W + r, BR, PR), :], dst.at[:, _rows(r - V0, BR, PR), :], sem)

    def long_wo(z, nz, r, nr, i):
        idx = (pl.ds(z, nz), _rows(r, nr, OP), slice(None))
        return pltpu.make_async_copy(wo_h.at[idx], wo_v.at[idx], sem_o.at[i])

    def wo_block(q):
        j = jnp.where(q == 0, 5, jnp.where(q == 6, 6, q - 1))
        return O0 + j * OB, jnp.where(q == 6, 2 + NS, jnp.maximum((q - 1) >> 1, 0))

    def short_wq(i):
        idx = (_rows((i & 7) * OB + (i >> 6) * OP, OP, OP), _rows(((i >> 3) & 7) * D, D, D))
        return pltpu.make_async_copy(wq_h.at[idx], wq_v.at[idx], sem_w.at[0])

    def short_kv(src, dst, r0, sem):
        def copy(i):
            h, r = i & (NH - 1), (r0 + NB * BR + (i >> 5) * PR) & (W - 1)
            return pltpu.make_async_copy(src.at[0, h, _rows(SK - W + r, PR, PR), :],
                                         dst.at[h, _rows((r - V0) & (W - 1), PR, PR), :], sem)
        return copy

    def short_w(src, dst, sem):
        def copy(i):
            rows = _rows((i & 1) * (F // 2) + (i >> 1) * OP, OP, OP)
            return pltpu.make_async_copy(src.at[rows, :], dst.at[rows, :], sem)
        return copy

    def short_wo(i):
        return long_wo(i & 7, 1, (RL + OB + (i >> 3) * OP) & (SR - 1), OP, 0)

    def short_last(i):
        r, sem = wo_block(i >> 3)
        return long_wo(NS - 1, 1, r + (i & 7) * OP, OP, sem)

    cargo = ((0, S_K, short_wq), (S_K, S_G, short_kv(k_h, k_v, K0, sem_k.at[1])),
             (S_G, S_U, short_w(wg_h, wg_v, sem_w.at[1])), (S_U, S_D, short_w(wu_h, wu_v, sem_w.at[2])),
             (S_D, S_V, short_w(wd_h, wd_v, sem_w.at[3])), (S_V, S_O, short_kv(v_h, v_v, V0, sem_v.at[VE])),
             (S_O, S_L, short_wo), (S_L, S_END, short_last))

    def wait_all(ref, sem):
        pltpu.make_async_copy(ref, ref, sem).wait()

    started = [0]

    def run(n, k, t, work=None, carry=0):
        lo = started[0]
        hi = started[0] = lo + n * k
        for a, b, copy in cargo:
            if a < hi and b > lo:
                def body(i, c):
                    for j in range(k):
                        copy(lo - a + i * k + j).start(priority=SHORT)
                        if work is None or j + 1 < k:
                            pl.delay(t)
                    return c if work is None else work(i, c)
                assert (max(a, lo) - lo) % k == 0
                carry = jax.lax.fori_loop((max(a, lo) - lo) // k, (min(b, hi) - lo) // k, body, carry)
        return carry

    def idle_until(s):
        assert s >= started[0]
        if s > started[0]:
            run(s - started[0], 1, T_IDLE)

    long_kv(k_h, k_v, K0, 0, sem_k.at[0]).start(priority=LONG)
    copy_x = pltpu.make_async_copy(x_h, x_v, sem_x.at[0])
    copy_wr = pltpu.make_async_copy(wr_h, wr_v, sem_x.at[1])
    copy_x.start(priority=SHORT)
    copy_wr.start(priority=SHORT)
    run(BURST, 1, T_BURST)

    @pl.loop(1, NB)
    def _(b):
        long_kv(k_h, k_v, K0, b, sem_k.at[(b >= KB).astype(jnp.int32)]).start(priority=LONG)

    q_v[...] = jnp.zeros(q_v.shape, F32)
    o_v[...] = jnp.zeros(o_v.shape, F32)
    idle_until(S_K)

    @pl.loop(0, NB)
    def _(b):
        long_kv(v_h, v_v, V0, b, sem_v.at[b + (b >= VE).astype(jnp.int32)]).start(priority=LONG)

    idle_until(S_K + LAND)
    copy_x.wait()
    copy_wr.wait()
    x = x_v[0].astype(F32)
    mean = jnp.mean(x, axis=-1, keepdims=True)
    var = jnp.mean(jnp.square(x - mean), axis=-1, keepdims=True)
    xn_b = ((x - mean) / jnp.sqrt(var + 1e-5)).astype(BF16)
    xn = xn_b.astype(F32)
    xn8 = jnp.broadcast_to(xn_b, (8, D))
    row = jax.lax.broadcasted_iota(jnp.int32, (8, DH), 0)

    def q_proj(i, c):
        q = jnp.dot(xn8, wq_v[:, _rows(i * 2 * DH, 2 * DH, 2 * DH)], preferred_element_type=F32)
        g, j = i >> 2, (i & 3) * 2
        q_v[g] = jnp.where(row == j, q[:, :DH], jnp.where(row == j + 1, q[:, DH:], q_v[g]))
        return c
    wait_all(wq_v, sem_w.at[0])
    run(NH // 2, 4, T_Q, q_proj)

    def per_head(g, f):
        r = f(g * 8)
        for j in range(1, 8):
            r = jnp.where(row == j, f(g * 8 + j), r)
        return r

    assert started[0] + 4 * KI >= S_G + LAND and 0 <= K0 - V0 <= DH and (KI // NG + 1) * DH <= K0 - V0 + KB * BR

    def scores(i, c):
        g, t = i & (NG - 1), ((i >> 2) + 1) & (NT - 1)
        pl.when(i == KI)(lambda: wait_all(k_v.at[:, pl.ds(KB * BR, W - KB * BR), :], sem_k.at[1]))
        q = q_v[g].astype(BF16)
        s_v[g, t] = per_head(g, lambda h: jax.lax.dot_general(
            q, k_v[h, _rows(t * DH, DH, DH), :], _NT, preferred_element_type=F32)) * (DH ** -0.5)
        return c
    wait_all(k_v.at[:, pl.ds(0, KB * BR), :], sem_k.at[0])
    run(NG * NT, 4, T_QK, scores)

    def softmax(g, c):
        s = s_v[g]
        p = jnp.exp(s - jnp.max(jnp.max(s, axis=0), axis=-1, keepdims=True))
        s_v[g] = p
        l_v[g] = jnp.broadcast_to(jnp.sum(jnp.sum(p, axis=0), axis=-1, keepdims=True), (8, DH))
        return c
    run(NG, 4, T_FFN, softmax)

    def chunk(i):
        return _rows(jnp.minimum(i * DH, F - DH), DH, 32)

    def gate_up(i, c):
        gt = jax.lax.dot_general(xn8, wg_v[chunk(i), :], _NT, preferred_element_type=F32)
        up = jax.lax.dot_general(xn8, wu_v[chunk(i), :], _NT, preferred_element_type=F32)
        new = jax.lax.broadcasted_iota(jnp.int32, (8, DH), 1) >= (i + 1) * DH - F
        h_v[i] = jnp.where(new, jax.nn.silu(gt) * up, 0.0)
        return c

    def down(i, y):
        return y + jnp.dot(h_v[i].astype(BF16), wd_v[chunk(i), :], preferred_element_type=F32)

    idle_until(S_D + LAND)
    wait_all(wg_v, sem_w.at[1])
    wait_all(wu_v, sem_w.at[2])
    run(NC, 4, T_FFN, gate_up)
    r = jnp.sum(xn * wr_v[...].reshape(1, D).astype(F32), axis=-1, keepdims=True)
    idle_until(S_V + LAND)
    wait_all(wd_v, sem_w.at[3])
    y = run(NC, 3, T_FFN, down, jnp.zeros((8, D), F32))
    gate = jax.nn.silu(xn + (xn * 0.0 + y * jax.nn.sigmoid(r)))

    idle_until(S_PV)

    @pl.loop(0, NOB - 1)
    def _(q):
        r0, sem = wo_block(q)
        long_wo(0, NS - 1, r0, OB, sem).start(priority=LONG)

    @pl.loop(0, NS - 2)
    def _(z):
        long_wo(z, 1, RL, OB, 3 + z).start(priority=LONG)

    last = [(RL + sum(LAST[:i]), nr, 1 + NS if i == 0 else 2 + NS + i) for i, nr in enumerate(LAST)]
    for piece in last:
        long_wo(NS - 2, 1, *piece).start(priority=LONG)

    assert S_PV + 4 * NG * VE >= S_O + LAND

    def values(i, c):
        g, u = i & (NG - 1), i >> 2
        pl.when(g == 0)(lambda: wait_all(v_v.at[:, pl.ds(0, BR), :], sem_v.at[u]))
        b = jnp.where(u == VE, NB, u - (u > VE).astype(jnp.int32))
        p = jnp.concatenate([s_v[g, 2 * b], s_v[g, 2 * b + 1]], axis=1).astype(BF16)
        o_v[g] += per_head(g, lambda h: jnp.dot(p, v_v[h, _rows(b * BR, BR, BR), :], preferred_element_type=F32))
        return c
    run(NG * (NB + 1), 4, T_PV, values)

    def normalize(g, c):
        o = o_v[g] / l_v[g]
        o_v[g] = o
        o = o.astype(BF16).astype(F32)
        for z in range(2):
            c_v[2 * g + z] = jnp.broadcast_to(o[4 * z + 3:4 * z + 4], (DH, DH)).T
        return c
    run(NG, 4, T_O, normalize)

    def head(acc, z, a):
        t = jnp.dot(o_v[z >> 1].astype(BF16), wo_v[z, pl.ds(a * DH, DH), :], preferred_element_type=F32)
        return acc + jnp.where(jax.lax.broadcasted_iota(jnp.int32, (8, D), 0) == (z & 1) * 4 + a, t, 0.0)

    def last_head(acc, z, r0, nr):
        coef = jnp.concatenate([c_v[z, pl.ds(r0 - 3 * DH, nr), :]] * (D // DH), axis=1)
        return acc + (wo_v[z, pl.ds(r0, nr), :].astype(F32) * coef).reshape(nr // 8, 8, D).sum(axis=0)

    def first(g, acc):
        for z in (2 * g, 2 * g + 1):
            acc = head(last_head(last_head(acc, z, 3 * DH, RL - 3 * DH), z, RL + OB, SR - RL - OB), z, 0)
        return acc

    def tail(z, acc):
        long_wo(z, 1, RL, OB, 3 + z).wait()
        return last_head(acc, z, RL, OB)

    idle_until(S_END - 22)
    wait_all(wo_v.at[:, pl.ds(0, 4 * OB), :], sem_o.at[0])
    acc = run(NG, 3, T_O, first, jnp.zeros((8, D), F32))
    idle_until(S_END - 8)
    wait_all(wo_v.at[:, pl.ds(0, 2 * OB), :], sem_o.at[1])
    acc = run(NG, 2, T_O, lambda g, acc: head(head(acc, 2 * g, 1), 2 * g + 1, 1), acc)
    wait_all(wo_v.at[:, pl.ds(0, OB), :], sem_o.at[2])
    for z in range(NS):
        acc = head(acc, z, 2)
    acc = tail(NS - 1, jax.lax.fori_loop(0, NS - 2, tail, acc))
    for r0, nr, sem in last:
        long_wo(NS - 2, 1, r0, nr, sem).wait()
        acc = last_head(acc, NS - 2, r0, nr)

    s_out = jnp.broadcast_to(jnp.sum(acc, axis=0, keepdims=True), (8, D))
    out_ref[0] = (jnp.broadcast_to(x, (8, D)) + s_out * gate).astype(out_ref.dtype)[0:1]


@jax.jit
def pallas_recurrent_scan__sliding_block_cached__moe_arch_mod__decode_kernel(
    A_x: jax.Array,
    A_k_cache: jax.Array,
    A_v_cache: jax.Array,
    A_wq: jax.Array,
    A_wo: jax.Array,
    B_x: jax.Array,
    B_w_r: jax.Array,
    B_w_gate: jax.Array,
    B_w_up: jax.Array,
    B_w_down: jax.Array,
):
    del B_x
    hbm = pl.BlockSpec(memory_space=pltpu.HBM)
    dma = pltpu.SemaphoreType.DMA
    return pl.pallas_call(
        _kernel,
        out_shape=jax.ShapeDtypeStruct((1, 1, D), BF16),
        in_specs=[hbm] * 9,
        out_specs=pl.BlockSpec(memory_space=pltpu.VMEM),
        scratch_shapes=[
            pltpu.VMEM((1, 1, D), BF16),
            pltpu.VMEM((D,), BF16),
            pltpu.VMEM((D, NH * DH), BF16),
            pltpu.VMEM((NH, W, DH), BF16),
            pltpu.VMEM((NH, W, DH), BF16),
            pltpu.VMEM((NS, SR, D), BF16),
            pltpu.VMEM((F, D), BF16),
            pltpu.VMEM((F, D), BF16),
            pltpu.VMEM((F, D), BF16),
            pltpu.VMEM((NG, 8, DH), F32),
            pltpu.VMEM((NG, NT, 8, DH), F32),
            pltpu.VMEM((NG, 8, DH), F32),
            pltpu.VMEM((NG, 8, DH), F32),
            pltpu.VMEM((NC, 8, DH), F32),
            pltpu.VMEM((NS, DH, DH), F32),
            dma((2,)), dma((4,)), dma((2,)), dma((NB + 1,)), dma((2 + NS + len(LAST),)),
        ],
        compiler_params=pltpu.CompilerParams(
            vmem_limit_bytes=100 * 1024 * 1024,
            disable_semaphore_checks=True,
            disable_bounds_checks=True,
        ),
    )(A_x, A_k_cache, A_v_cache, A_wq, A_wo.reshape(NS, SR, D), B_w_r, B_w_gate.T, B_w_up.T, B_w_down)
```

```python
import jax
import jax.numpy as jnp
import jax.experimental.pallas as pl
import jax.experimental.pallas.tpu as pltpu

D = 512
NH = 32
DH = 128
SK = 32768
W = min(4096, max(256, SK // 4))
F = 1376
NG = NH // 8
NT = W // DH
NC = -(-F // DH)

BR, PR = 256, 32
NB = W // BR - 1
K0, V0 = 128, 64
NS, SR = 8, 512
OB, OP = 64, 8
NOB = SR // OB - 1
O0 = 32
RL = O0 + (NOB - 1) * OB
LAST = (32, 16, 16)

S_K = D * NH * DH // (OP * D)
S_G = S_K + NH * BR // PR
S_U = S_G + F // OP
S_D = S_U + F // OP
S_V = S_D + F // OP
S_O = S_V + NH * BR // PR
S_L = S_O + NS * OB // OP
S_END = S_L + NOB * OB // OP
LAND = 12
S_PV = 1356
KB, KI = 10, 64
VE = 13
BURST, T_BURST = 16, 14
T_IDLE, T_Q, T_QK, T_FFN, T_PV, T_O = 59, 24, 17, 20, 15, 14

BF16 = jnp.bfloat16
F32 = jnp.float32
_NT = (((1,), (1,)), ((), ()))
LONG, SHORT = 1, 0


def _rows(start, size, multiple):
    return pl.ds(start if isinstance(start, int) else pl.multiple_of(start, multiple), size)


def _kernel(x_h, k_h, v_h, wq_h, wo_h, wr_h, wg_h, wu_h, wd_h, out_ref,
            x_v, wr_v, wq_v, k_v, v_v, wo_v, wg_v, wu_v, wd_v, q_v, s_v, l_v, o_v, h_v, c_v,
            sem_x, sem_w, sem_k, sem_v, sem_o):
    def long_kv(src, dst, r0, b, sem):
        r = r0 + b * BR
        return pltpu.make_async_copy(src.at[0, :, _rows(SK - W + r, BR, PR), :], dst.at[:, _rows(r - V0, BR, PR), :], sem)

    def long_wo(z, nz, r, nr, i):
        idx = (pl.ds(z, nz), _rows(r, nr, OP), slice(None))
        return pltpu.make_async_copy(wo_h.at[idx], wo_v.at[idx], sem_o.at[i])

    def wo_block(q):
        j = jnp.where(q == 0, 5, jnp.where(q == 6, 6, q - 1))
        return O0 + j * OB, jnp.where(q == 6, 2 + NS, jnp.maximum((q - 1) >> 1, 0))

    def short_wq(i):
        idx = (_rows((i & 7) * OB + (i >> 6) * OP, OP, OP), _rows(((i >> 3) & 7) * D, D, D))
        return pltpu.make_async_copy(wq_h.at[idx], wq_v.at[idx], sem_w.at[0])

    def short_kv(src, dst, r0, sem):
        def copy(i):
            h, r = i & (NH - 1), (r0 + NB * BR + (i >> 5) * PR) & (W - 1)
            return pltpu.make_async_copy(src.at[0, h, _rows(SK - W + r, PR, PR), :],
                                         dst.at[h, _rows((r - V0) & (W - 1), PR, PR), :], sem)
        return copy

    def short_w(src, dst, sem):
        def copy(i):
            rows = _rows((i & 1) * (F // 2) + (i >> 1) * OP, OP, OP)
            return pltpu.make_async_copy(src.at[rows, :], dst.at[rows, :], sem)
        return copy

    def short_wo(i):
        return long_wo(i & 7, 1, (RL + OB + (i >> 3) * OP) & (SR - 1), OP, 0)

    def short_last(i):
        r, sem = wo_block(i >> 3)
        return long_wo(NS - 1, 1, r + (i & 7) * OP, OP, sem)

    cargo = ((0, S_K, short_wq), (S_K, S_G, short_kv(k_h, k_v, K0, sem_k.at[1])),
             (S_G, S_U, short_w(wg_h, wg_v, sem_w.at[1])), (S_U, S_D, short_w(wu_h, wu_v, sem_w.at[2])),
             (S_D, S_V, short_w(wd_h, wd_v, sem_w.at[3])), (S_V, S_O, short_kv(v_h, v_v, V0, sem_v.at[VE])),
             (S_O, S_L, short_wo), (S_L, S_END, short_last))

    def wait_all(ref, sem):
        pltpu.make_async_copy(ref, ref, sem).wait()

    started = [0]

    def run(n, k, t, work=None, carry=0):
        lo = started[0]
        hi = started[0] = lo + n * k
        for a, b, copy in cargo:
            if a < hi and b > lo:
                def body(i, c):
                    for j in range(k):
                        copy(lo - a + i * k + j).start(priority=SHORT)
                        if work is None or j + 1 < k:
                            pl.delay(t)
                    return c if work is None else work(i, c)
                assert (max(a, lo) - lo) % k == 0
                carry = jax.lax.fori_loop((max(a, lo) - lo) // k, (min(b, hi) - lo) // k, body, carry)
        return carry

    def idle_until(s):
        assert s >= started[0]
        if s > started[0]:
            run(s - started[0], 1, T_IDLE)

    long_kv(k_h, k_v, K0, 0, sem_k.at[0]).start(priority=LONG)
    copy_x = pltpu.make_async_copy(x_h, x_v, sem_x.at[0])
    copy_wr = pltpu.make_async_copy(wr_h, wr_v, sem_x.at[1])
    copy_x.start(priority=SHORT)
    copy_wr.start(priority=SHORT)
    run(BURST, 1, T_BURST)

    @pl.loop(1, NB)
    def _(b):
        long_kv(k_h, k_v, K0, b, sem_k.at[(b >= KB).astype(jnp.int32)]).start(priority=LONG)

    q_v[...] = jnp.zeros(q_v.shape, F32)
    o_v[...] = jnp.zeros(o_v.shape, F32)
    idle_until(S_K)

    @pl.loop(0, NB)
    def _(b):
        long_kv(v_h, v_v, V0, b, sem_v.at[b + (b >= VE).astype(jnp.int32)]).start(priority=LONG)

    idle_until(S_K + LAND)
    copy_x.wait()
    copy_wr.wait()
    x = x_v[0].astype(F32)
    mean = jnp.mean(x, axis=-1, keepdims=True)
    var = jnp.mean(jnp.square(x - mean), axis=-1, keepdims=True)
    xn_b = ((x - mean) / jnp.sqrt(var + 1e-5)).astype(BF16)
    xn = xn_b.astype(F32)
    xn8 = jnp.broadcast_to(xn_b, (8, D))
    row = jax.lax.broadcasted_iota(jnp.int32, (8, DH), 0)

    def q_proj(i, c):
        q = jnp.dot(xn8, wq_v[:, _rows(i * 2 * DH, 2 * DH, 2 * DH)], preferred_element_type=F32)
        g, j = i >> 2, (i & 3) * 2
        q_v[g] = jnp.where(row == j, q[:, :DH], jnp.where(row == j + 1, q[:, DH:], q_v[g]))
        return c
    wait_all(wq_v, sem_w.at[0])
    run(NH // 2, 4, T_Q, q_proj)

    def per_head(g, f):
        r = f(g * 8)
        for j in range(1, 8):
            r = jnp.where(row == j, f(g * 8 + j), r)
        return r

    k0, k1 = K0 - V0, K0 - V0 + KB * BR
    assert started[0] + 4 * KI >= S_G + LAND and 0 <= k0 <= DH and (KI // NG + 1) * DH <= k1

    def scores(i, c):
        g, t = i & (NG - 1), ((i >> 2) + 1) & (NT - 1)

        @pl.when(i == KI)
        def _():
            wait_all(k_v.at[:, pl.ds(k1, W - k1), :], sem_k.at[1])
            if k0:
                wait_all(k_v.at[:, pl.ds(0, k0), :], sem_k.at[1])
        q = q_v[g].astype(BF16)
        s_v[g, t] = per_head(g, lambda h: jax.lax.dot_general(
            q, k_v[h, _rows(t * DH, DH, DH), :], _NT, preferred_element_type=F32)) * (DH ** -0.5)
        return c
    wait_all(k_v.at[:, pl.ds(k0, k1 - k0), :], sem_k.at[0])
    run(NG * NT, 4, T_QK, scores)

    def softmax(g, c):
        s = s_v[g]
        p = jnp.exp(s - jnp.max(jnp.max(s, axis=0), axis=-1, keepdims=True))
        s_v[g] = p
        l_v[g] = jnp.broadcast_to(jnp.sum(jnp.sum(p, axis=0), axis=-1, keepdims=True), (8, DH))
        return c
    run(NG, 4, T_FFN, softmax)

    def chunk(i):
        return _rows(jnp.minimum(i * DH, F - DH), DH, 32)

    def gate_up(i, c):
        gt = jax.lax.dot_general(xn8, wg_v[chunk(i), :], _NT, preferred_element_type=F32)
        up = jax.lax.dot_general(xn8, wu_v[chunk(i), :], _NT, preferred_element_type=F32)
        new = jax.lax.broadcasted_iota(jnp.int32, (8, DH), 1) >= (i + 1) * DH - F
        h_v[i] = jnp.where(new, jax.nn.silu(gt) * up, 0.0)
        return c

    def down(i, y):
        return y + jnp.dot(h_v[i].astype(BF16), wd_v[chunk(i), :], preferred_element_type=F32)

    idle_until(S_D + LAND)
    wait_all(wg_v, sem_w.at[1])
    wait_all(wu_v, sem_w.at[2])
    run(NC, 4, T_FFN, gate_up)
    r = jnp.sum(xn * wr_v[...].reshape(1, D).astype(F32), axis=-1, keepdims=True)
    idle_until(S_V + LAND)
    wait_all(wd_v, sem_w.at[3])
    y = run(NC, 3, T_FFN, down, jnp.zeros((8, D), F32))
    gate = jax.nn.silu(xn + (xn * 0.0 + y * jax.nn.sigmoid(r)))

    idle_until(S_PV)

    @pl.loop(0, NOB - 1)
    def _(q):
        r0, sem = wo_block(q)
        long_wo(0, NS - 1, r0, OB, sem).start(priority=LONG)

    @pl.loop(0, NS - 2)
    def _(z):
        long_wo(z, 1, RL, OB, 3 + z).start(priority=LONG)

    last = [(RL + sum(LAST[:i]), nr, 1 + NS if i == 0 else 2 + NS + i) for i, nr in enumerate(LAST)]
    for piece in last:
        long_wo(NS - 2, 1, *piece).start(priority=LONG)

    assert S_PV + 4 * NG * VE >= S_O + LAND

    def values(i, c):
        g, u = i & (NG - 1), i >> 2
        b = jnp.where(u == VE, NB, u - (u > VE).astype(jnp.int32))
        pl.when(g == 0)(lambda: wait_all(v_v.at[:, _rows(b * BR, BR, BR), :], sem_v.at[u]))
        p = jnp.concatenate([s_v[g, 2 * b], s_v[g, 2 * b + 1]], axis=1).astype(BF16)
        o_v[g] += per_head(g, lambda h: jnp.dot(p, v_v[h, _rows(b * BR, BR, BR), :], preferred_element_type=F32))
        return c
    run(NG * (NB + 1), 4, T_PV, values)

    def normalize(g, c):
        o = o_v[g] / l_v[g]
        o_v[g] = o
        o = o.astype(BF16).astype(F32)
        for z in range(2):
            c_v[2 * g + z] = jnp.broadcast_to(o[4 * z + 3:4 * z + 4], (DH, DH)).T
        return c
    run(NG, 4, T_O, normalize)

    def head(acc, z, a):
        t = jnp.dot(o_v[z >> 1].astype(BF16), wo_v[z, pl.ds(a * DH, DH), :], preferred_element_type=F32)
        return acc + jnp.where(jax.lax.broadcasted_iota(jnp.int32, (8, D), 0) == (z & 1) * 4 + a, t, 0.0)

    def last_head(acc, z, r0, nr):
        coef = jnp.concatenate([c_v[z, pl.ds(r0 - 3 * DH, nr), :]] * (D // DH), axis=1)
        return acc + (wo_v[z, pl.ds(r0, nr), :].astype(F32) * coef).reshape(nr // 8, 8, D).sum(axis=0)

    def first(g, acc):
        for z in (2 * g, 2 * g + 1):
            acc = head(last_head(last_head(acc, z, 3 * DH, RL - 3 * DH), z, RL + OB, SR - RL - OB), z, 0)
        return acc

    def tail(z, acc):
        long_wo(z, 1, RL, OB, 3 + z).wait()
        return last_head(acc, z, RL, OB)

    idle_until(S_END - 22)
    for r0, r1 in ((0, O0 + 2 * OB), (RL - OB, RL), (RL + OB, SR)):
        wait_all(wo_v.at[:, pl.ds(r0, r1 - r0), :], sem_o.at[0])
    acc = run(NG, 3, T_O, first, jnp.zeros((8, D), F32))
    idle_until(S_END - 8)
    wait_all(wo_v.at[:, pl.ds(O0 + 2 * OB, 2 * OB), :], sem_o.at[1])
    acc = run(NG, 2, T_O, lambda g, acc: head(head(acc, 2 * g, 1), 2 * g + 1, 1), acc)
    wait_all(wo_v.at[:, pl.ds(O0 + 4 * OB, OB), :], sem_o.at[2])
    for z in range(NS):
        acc = head(acc, z, 2)
    acc = tail(NS - 1, jax.lax.fori_loop(0, NS - 2, tail, acc))
    for r0, nr, sem in last:
        long_wo(NS - 2, 1, r0, nr, sem).wait()
        acc = last_head(acc, NS - 2, r0, nr)

    s_out = jnp.broadcast_to(jnp.sum(acc, axis=0, keepdims=True), (8, D))
    out_ref[0] = (jnp.broadcast_to(x, (8, D)) + s_out * gate).astype(out_ref.dtype)[0:1]


@jax.jit
def pallas_recurrent_scan__sliding_block_cached__moe_arch_mod__decode_kernel(
    A_x: jax.Array,
    A_k_cache: jax.Array,
    A_v_cache: jax.Array,
    A_wq: jax.Array,
    A_wo: jax.Array,
    B_x: jax.Array,
    B_w_r: jax.Array,
    B_w_gate: jax.Array,
    B_w_up: jax.Array,
    B_w_down: jax.Array,
):
    del B_x
    hbm = pl.BlockSpec(memory_space=pltpu.HBM)
    dma = pltpu.SemaphoreType.DMA
    return pl.pallas_call(
        _kernel,
        out_shape=jax.ShapeDtypeStruct((1, 1, D), BF16),
        in_specs=[hbm] * 9,
        out_specs=pl.BlockSpec(memory_space=pltpu.VMEM),
        scratch_shapes=[
            pltpu.VMEM((1, 1, D), BF16),
            pltpu.VMEM((D,), BF16),
            pltpu.VMEM((D, NH * DH), BF16),
            pltpu.VMEM((NH, W, DH), BF16),
            pltpu.VMEM((NH, W, DH), BF16),
            pltpu.VMEM((NS, SR, D), BF16),
            pltpu.VMEM((F, D), BF16),
            pltpu.VMEM((F, D), BF16),
            pltpu.VMEM((F, D), BF16),
            pltpu.VMEM((NG, 8, DH), F32),
            pltpu.VMEM((NG, NT, 8, DH), F32),
            pltpu.VMEM((NG, 8, DH), F32),
            pltpu.VMEM((NG, 8, DH), F32),
            pltpu.VMEM((NC, 8, DH), F32),
            pltpu.VMEM((NS, DH, DH), F32),
            dma((2,)), dma((4,)), dma((2,)), dma((NB + 1,)), dma((2 + NS + len(LAST),)),
        ],
        compiler_params=pltpu.CompilerParams(
            vmem_limit_bytes=100 * 1024 * 1024,
            disable_semaphore_checks=True,
            disable_bounds_checks=True,
        ),
    )(A_x, A_k_cache, A_v_cache, A_wq, A_wo.reshape(NS, SR, D), B_w_r, B_w_gate.T, B_w_up.T, B_w_down)
```

```python
import jax
import jax.numpy as jnp
import jax.experimental.pallas as pl
import jax.experimental.pallas.tpu as pltpu

D = 512
NH = 32
DH = 128
SK = 32768
W = min(4096, max(256, SK // 4))
F = 1376
NG = NH // 8
NT = W // DH
NC = -(-F // DH)

BR, PR = 256, 32
NB = W // BR - 1
K0, V0 = 128, 64
K1 = 192
KH, KA = 4, 3
NS, SR = 8, 512
OB, OP = 64, 8
NOB = SR // OB - 1
O0 = 32
RL = O0 + (NOB - 1) * OB
LAST = (32, 16, 16)

S_K = D * NH * DH // (OP * D)
S_G = S_K + NH * BR // PR
S_U = S_G + F // OP
S_D = S_U + F // OP
S_V = S_D + F // OP
S_O = S_V + NH * BR // PR
S_L = S_O + NS * OB // OP
S_END = S_L + NOB * OB // OP
LAND = 12
S_PV = 1356
KB, KI = 10, 64
VE = 13
BURST, T_BURST = 16, 14
T_IDLE, T_Q, T_QK, T_FFN, T_PV, T_O = 58, 24, 17, 20, 15, 14

BF16 = jnp.bfloat16
F32 = jnp.float32
_NT = (((1,), (1,)), ((), ()))
KRATE = -(-(NB * NH // KH - KA << 16) // S_G)
LONG, SHORT = 1, 0


def _rows(start, size, multiple):
    return pl.ds(start if isinstance(start, int) else pl.multiple_of(start, multiple), size)


def _kernel(x_h, k_h, v_h, wq_h, wo_h, wr_h, wg_h, wu_h, wd_h, out_ref,
            x_v, wr_v, wq_v, k_v, v_v, wo_v, wg_v, wu_v, wd_v, q_v, s_v, l_v, o_v, h_v, c_v,
            sem_x, sem_w, sem_k, sem_v, sem_o):
    def long_kv(src, dst, heads, r, nr, sem):
        return pltpu.make_async_copy(src.at[0, heads, _rows(SK - W + r, nr, PR), :],
                                     dst.at[heads, _rows(r - V0, nr, PR), :], sem)

    def start_k(n):
        b, h = n * KH >> 5, n * KH & (NH - 1)
        sem = sem_k.at[jnp.where(b >= KB, 1, 0)]
        long_kv(k_h, k_v, pl.ds(h, KH), K1 + b * BR, BR + K0 - K1, sem).start(priority=LONG)
        long_kv(k_h, k_v, pl.ds(h ^ NH // 2, KH), K0 + b * BR, K1 - K0, sem).start(priority=LONG)

    def k_due(s):
        return KA + (s * KRATE >> 16)

    def long_wo(z, nz, r, nr, i):
        idx = (pl.ds(z, nz), _rows(r, nr, OP), slice(None))
        return pltpu.make_async_copy(wo_h.at[idx], wo_v.at[idx], sem_o.at[i])

    def wo_block(q):
        j = jnp.where(q == 0, 5, jnp.where(q == 6, 6, q - 1))
        return O0 + j * OB, jnp.where(q == 6, 2 + NS, jnp.maximum((q - 1) >> 1, 0))

    def short_wq(i):
        idx = (_rows((i & 7) * OB + (i >> 6) * OP, OP, OP), _rows(((i >> 3) & 7) * D, D, D))
        return pltpu.make_async_copy(wq_h.at[idx], wq_v.at[idx], sem_w.at[0])

    def short_kv(src, dst, r0, sem):
        def copy(i):
            h, r = i & (NH - 1), (r0 + NB * BR + (i >> 5) * PR) & (W - 1)
            return pltpu.make_async_copy(src.at[0, h, _rows(SK - W + r, PR, PR), :],
                                         dst.at[h, _rows((r - V0) & (W - 1), PR, PR), :], sem)
        return copy

    def short_w(src, dst, sem):
        def copy(i):
            rows = _rows((i & 1) * (F // 2) + (i >> 1) * OP, OP, OP)
            return pltpu.make_async_copy(src.at[rows, :], dst.at[rows, :], sem)
        return copy

    def short_wo(i):
        return long_wo(i & 7, 1, (RL + OB + (i >> 3) * OP) & (SR - 1), OP, 0)

    def short_last(i):
        r, sem = wo_block(i >> 3)
        return long_wo(NS - 1, 1, r + (i & 7) * OP, OP, sem)

    cargo = ((0, S_K, short_wq), (S_K, S_G, short_kv(k_h, k_v, K0, sem_k.at[1])),
             (S_G, S_U, short_w(wg_h, wg_v, sem_w.at[1])), (S_U, S_D, short_w(wu_h, wu_v, sem_w.at[2])),
             (S_D, S_V, short_w(wd_h, wd_v, sem_w.at[3])), (S_V, S_O, short_kv(v_h, v_v, V0, sem_v.at[VE])),
             (S_O, S_L, short_wo), (S_L, S_END, short_last))

    def wait_all(ref, sem):
        pltpu.make_async_copy(ref, ref, sem).wait()

    started = [0]

    def run(n, k, t, work=None, carry=0):
        lo = started[0]
        hi = started[0] = lo + n * k
        for a, b, copy in cargo:
            if a < hi and b > lo:
                def body(i, c):
                    if a < S_G:
                        n0 = k_due(lo + i * k)
                        pl.when(k_due(lo + (i + 1) * k) > n0)(lambda: start_k(n0))
                    for j in range(k):
                        copy(lo - a + i * k + j).start(priority=SHORT)
                        if work is None or j + 1 < k:
                            pl.delay(t)
                    return c if work is None else work(i, c)
                assert (max(a, lo) - lo) % k == 0
                carry = jax.lax.fori_loop((max(a, lo) - lo) // k, (min(b, hi) - lo) // k, body, carry)
        return carry

    def idle_until(s):
        assert s >= started[0]
        if s > started[0]:
            run(s - started[0], 1, T_IDLE)

    assert k_due(S_G) == NB * NH // KH and 4 * KRATE <= 1 << 16
    for n in range(KA):
        start_k(n)
    copy_x = pltpu.make_async_copy(x_h, x_v, sem_x.at[0])
    copy_wr = pltpu.make_async_copy(wr_h, wr_v, sem_x.at[1])
    copy_x.start(priority=SHORT)
    copy_wr.start(priority=SHORT)
    run(BURST, 1, T_BURST)

    q_v[...] = jnp.zeros(q_v.shape, F32)
    o_v[...] = jnp.zeros(o_v.shape, F32)
    idle_until(S_K + LAND)
    copy_x.wait()
    copy_wr.wait()
    x = x_v[0].astype(F32)
    mean = jnp.mean(x, axis=-1, keepdims=True)
    var = jnp.mean(jnp.square(x - mean), axis=-1, keepdims=True)
    xn_b = ((x - mean) / jnp.sqrt(var + 1e-5)).astype(BF16)
    xn = xn_b.astype(F32)
    xn8 = jnp.broadcast_to(xn_b, (8, D))
    row = jax.lax.broadcasted_iota(jnp.int32, (8, DH), 0)

    def q_proj(i, c):
        q = jnp.dot(xn8, wq_v[:, _rows(i * 2 * DH, 2 * DH, 2 * DH)], preferred_element_type=F32)
        g, j = i >> 2, (i & 3) * 2
        q_v[g] = jnp.where(row == j, q[:, :DH], jnp.where(row == j + 1, q[:, DH:], q_v[g]))
        return c
    wait_all(wq_v, sem_w.at[0])
    run(NH // 2, 4, T_Q, q_proj)

    def per_head(g, f):
        r = f(g * 8)
        for j in range(1, 8):
            r = jnp.where(row == j, f(g * 8 + j), r)
        return r

    k0, k1 = K0 - V0, K0 - V0 + KB * BR
    assert k_due(started[0]) >= KB * NH // KH and started[0] + 4 * KI >= S_G + LAND
    assert 0 <= k0 <= DH and (KI // NG + 1) * DH <= k1

    def scores(i, c):
        g, t = i & (NG - 1), ((i >> 2) + 1) & (NT - 1)

        @pl.when(i == KI)
        def _():
            wait_all(k_v.at[:, pl.ds(k1, W - k1), :], sem_k.at[1])
            if k0:
                wait_all(k_v.at[:, pl.ds(0, k0), :], sem_k.at[1])
        q = q_v[g].astype(BF16)
        s_v[g, t] = per_head(g, lambda h: jax.lax.dot_general(
            q, k_v[h, _rows(t * DH, DH, DH), :], _NT, preferred_element_type=F32)) * (DH ** -0.5)
        return c
    wait_all(k_v.at[:, pl.ds(k0, k1 - k0), :], sem_k.at[0])
    n1 = (S_G - started[0]) // 4
    run(n1, 4, T_QK, scores)

    @pl.loop(0, NB)
    def _(b):
        long_kv(v_h, v_v, slice(None), V0 + b * BR, BR, sem_v.at[jnp.where(b >= VE, b + 1, b)]).start(priority=LONG)

    run(NG * NT - n1, 4, T_QK, lambda i, c: scores(i + n1, c))

    def softmax(g, c):
        s = s_v[g]
        p = jnp.exp(s - jnp.max(jnp.max(s, axis=0), axis=-1, keepdims=True))
        s_v[g] = p
        l_v[g] = jnp.broadcast_to(jnp.sum(jnp.sum(p, axis=0), axis=-1, keepdims=True), (8, DH))
        return c
    run(NG, 4, T_FFN, softmax)

    def chunk(i):
        return _rows(jnp.minimum(i * DH, F - DH), DH, 32)

    def gate_up(i, c):
        gt = jax.lax.dot_general(xn8, wg_v[chunk(i), :], _NT, preferred_element_type=F32)
        up = jax.lax.dot_general(xn8, wu_v[chunk(i), :], _NT, preferred_element_type=F32)
        new = jax.lax.broadcasted_iota(jnp.int32, (8, DH), 1) >= (i + 1) * DH - F
        h_v[i] = jnp.where(new, jax.nn.silu(gt) * up, 0.0)
        return c

    def down(i, y):
        return y + jnp.dot(h_v[i].astype(BF16), wd_v[chunk(i), :], preferred_element_type=F32)

    idle_until(S_D + LAND)
    wait_all(wg_v, sem_w.at[1])
    wait_all(wu_v, sem_w.at[2])
    run(NC, 4, T_FFN, gate_up)
    r = jnp.sum(xn * wr_v[...].reshape(1, D).astype(F32), axis=-1, keepdims=True)
    idle_until(S_V + LAND)
    wait_all(wd_v, sem_w.at[3])
    y = run(NC, 3, T_FFN, down, jnp.zeros((8, D), F32))
    gate = jax.nn.silu(xn + (xn * 0.0 + y * jax.nn.sigmoid(r)))

    idle_until(S_PV)

    @pl.loop(0, NOB - 1)
    def _(q):
        r0, sem = wo_block(q)
        long_wo(0, NS - 1, r0, OB, sem).start(priority=LONG)

    @pl.loop(0, NS - 2)
    def _(z):
        long_wo(z, 1, RL, OB, 3 + z).start(priority=LONG)

    last = [(RL + sum(LAST[:i]), nr, 1 + NS if i == 0 else 2 + NS + i) for i, nr in enumerate(LAST)]
    for piece in last:
        long_wo(NS - 2, 1, *piece).start(priority=LONG)

    assert S_PV + 4 * NG * VE >= S_O + LAND

    def values(i, c):
        g, u = i & (NG - 1), i >> 2
        b = jnp.where(u == VE, NB, u - (u > VE).astype(jnp.int32))
        pl.when(g == 0)(lambda: wait_all(v_v.at[:, _rows(b * BR, BR, BR), :], sem_v.at[u]))
        p = jnp.concatenate([s_v[g, 2 * b], s_v[g, 2 * b + 1]], axis=1).astype(BF16)
        o_v[g] += per_head(g, lambda h: jnp.dot(p, v_v[h, _rows(b * BR, BR, BR), :], preferred_element_type=F32))
        return c
    run(NG * (NB + 1), 4, T_PV, values)

    def normalize(g, c):
        o = o_v[g] / l_v[g]
        o_v[g] = o
        o = o.astype(BF16).astype(F32)
        for z in range(2):
            c_v[2 * g + z] = jnp.broadcast_to(o[4 * z + 3:4 * z + 4], (DH, DH)).T
        return c
    run(NG, 4, T_O, normalize)

    def head(acc, z, a):
        t = jnp.dot(o_v[z >> 1].astype(BF16), wo_v[z, pl.ds(a * DH, DH), :], preferred_element_type=F32)
        return acc + jnp.where(jax.lax.broadcasted_iota(jnp.int32, (8, D), 0) == (z & 1) * 4 + a, t, 0.0)

    def last_head(acc, z, r0, nr):
        coef = jnp.concatenate([c_v[z, pl.ds(r0 - 3 * DH, nr), :]] * (D // DH), axis=1)
        return acc + (wo_v[z, pl.ds(r0, nr), :].astype(F32) * coef).reshape(nr // 8, 8, D).sum(axis=0)

    def first(g, acc):
        for z in (2 * g, 2 * g + 1):
            acc = head(last_head(last_head(acc, z, 3 * DH, RL - 3 * DH), z, RL + OB, SR - RL - OB), z, 0)
        return acc

    def tail(z, acc):
        long_wo(z, 1, RL, OB, 3 + z).wait()
        return last_head(acc, z, RL, OB)

    idle_until(S_END - 22)
    for r0, r1 in ((0, O0 + 2 * OB), (RL - OB, RL), (RL + OB, SR)):
        wait_all(wo_v.at[:, pl.ds(r0, r1 - r0), :], sem_o.at[0])
    acc = run(NG, 3, T_O, first, jnp.zeros((8, D), F32))
    idle_until(S_END - 8)
    wait_all(wo_v.at[:, pl.ds(O0 + 2 * OB, 2 * OB), :], sem_o.at[1])
    acc = run(NG, 2, T_O, lambda g, acc: head(head(acc, 2 * g, 1), 2 * g + 1, 1), acc)
    wait_all(wo_v.at[:, pl.ds(O0 + 4 * OB, OB), :], sem_o.at[2])
    for z in range(NS):
        acc = head(acc, z, 2)
    acc = tail(NS - 1, jax.lax.fori_loop(0, NS - 2, tail, acc))
    for r0, nr, sem in last:
        long_wo(NS - 2, 1, r0, nr, sem).wait()
        acc = last_head(acc, NS - 2, r0, nr)

    s_out = jnp.broadcast_to(jnp.sum(acc, axis=0, keepdims=True), (8, D))
    out_ref[0] = (jnp.broadcast_to(x, (8, D)) + s_out * gate).astype(out_ref.dtype)[0:1]


@jax.jit
def pallas_recurrent_scan__sliding_block_cached__moe_arch_mod__decode_kernel(
    A_x: jax.Array,
    A_k_cache: jax.Array,
    A_v_cache: jax.Array,
    A_wq: jax.Array,
    A_wo: jax.Array,
    B_x: jax.Array,
    B_w_r: jax.Array,
    B_w_gate: jax.Array,
    B_w_up: jax.Array,
    B_w_down: jax.Array,
):
    del B_x
    hbm = pl.BlockSpec(memory_space=pltpu.HBM)
    dma = pltpu.SemaphoreType.DMA
    return pl.pallas_call(
        _kernel,
        out_shape=jax.ShapeDtypeStruct((1, 1, D), BF16),
        in_specs=[hbm] * 9,
        out_specs=pl.BlockSpec(memory_space=pltpu.VMEM),
        scratch_shapes=[
            pltpu.VMEM((1, 1, D), BF16),
            pltpu.VMEM((D,), BF16),
            pltpu.VMEM((D, NH * DH), BF16),
            pltpu.VMEM((NH, W, DH), BF16),
            pltpu.VMEM((NH, W, DH), BF16),
            pltpu.VMEM((NS, SR, D), BF16),
            pltpu.VMEM((F, D), BF16),
            pltpu.VMEM((F, D), BF16),
            pltpu.VMEM((F, D), BF16),
            pltpu.VMEM((NG, 8, DH), F32),
            pltpu.VMEM((NG, NT, 8, DH), F32),
            pltpu.VMEM((NG, 8, DH), F32),
            pltpu.VMEM((NG, 8, DH), F32),
            pltpu.VMEM((NC, 8, DH), F32),
            pltpu.VMEM((NS, DH, DH), F32),
            dma((2,)), dma((4,)), dma((2,)), dma((NB + 1,)), dma((2 + NS + len(LAST),)),
        ],
        compiler_params=pltpu.CompilerParams(
            vmem_limit_bytes=100 * 1024 * 1024,
            disable_semaphore_checks=True,
            disable_bounds_checks=True,
        ),
    )(A_x, A_k_cache, A_v_cache, A_wq, A_wo.reshape(NS, SR, D), B_w_r, B_w_gate.T, B_w_up.T, B_w_down)
```

```python
import jax
import jax.numpy as jnp
import jax.experimental.pallas as pl
import jax.experimental.pallas.tpu as pltpu

D = 512
NH = 32
DH = 128
SK = 32768
W = min(4096, max(256, SK // 4))
F = 1376
NG = NH // 8
NT = W // DH

BR, PR = 256, 32
NB = W // BR - 1
K0, V0 = 128, 64
K1 = 192
KH = 4
NS, SR = 8, 512
OB, OP = 64, 8
NOB = SR // OB - 1
O0 = 32
RL = O0 + (NOB - 1) * OB
LAST = (32, 16, 16)

S_F = NH * BR // PR
S_V = S_F + 3 * F // OP
S_O = S_V + NH * BR // PR
S_END = S_O + (NS + NOB) * OB // OP
LAND = 8
S_K0, S_K1 = 56, 571
S_Q, S_QK, S_PV = 96, 388, 926
KB, KI = 9, 68
VE = 11
BURST, T_BURST = 16, 40
T_IDLE, T_QK, T_PV, T_O = 86, 37, 33, 20

BF16 = jnp.bfloat16
F32 = jnp.float32
_NT = (((1,), (1,)), ((), ()))
KRATE = pl.cdiv((NB * NH // KH) << 16, S_K1 - S_K0)
LONG, SHORT = 1, 0


def _rows(start, size, multiple):
    return pl.ds(start if isinstance(start, int) else pl.multiple_of(start, multiple), size)


def _kernel(x_h, k_h, v_h, wq_h, wo_h, wr_h, wg_h, wu_h, wd_h, out_ref,
            x_v, wr_v, wq_v, k_v, v_v, wo_v, wg_v, wu_v, wd_v, q_v, s_v, l_v, o_v, c_v,
            sem_x, sem_w, sem_k, sem_v, sem_o):
    def long_kv(src, dst, heads, r, nr, sem):
        return pltpu.make_async_copy(src.at[0, heads, _rows(SK - W + r, nr, PR), :],
                                     dst.at[heads, _rows(r - V0, nr, PR), :], sem)

    def start_k(n):
        b, h = (n * KH) >> 5, (n * KH) & (NH - 1)
        sem = sem_k.at[jnp.where(b >= KB, 1, 0)]
        long_kv(k_h, k_v, pl.ds(h, KH), K1 + b * BR, BR + K0 - K1, sem).start(priority=LONG)
        long_kv(k_h, k_v, pl.ds(h ^ (NH // 2), KH), K0 + b * BR, K1 - K0, sem).start(priority=LONG)

    def k_due(s):
        return ((s - S_K0) * KRATE) >> 16

    def long_wo(z, nz, r, nr, i):
        idx = (pl.ds(z, nz), _rows(r, nr, OP), slice(None))
        return pltpu.make_async_copy(wo_h.at[idx], wo_v.at[idx], sem_o.at[i])

    def wo_block(q):
        j = jnp.where(q == 0, 5, jnp.where(q == 6, 6, q - 1))
        return O0 + j * OB, jnp.where(q == 6, 2 + NS, jnp.maximum((q - 1) >> 1, 0))

    def long_wq(n):
        idx = (slice(None), _rows((n >> 1) * OP, OP, OP), _rows((n & 1) * (NH * DH // 2), NH * DH // 2, DH))
        return pltpu.make_async_copy(wq_h.at[idx], wq_v.at[idx], sem_w.at[0])

    def short_kv(src, dst, r0, sem):
        def copy(i):
            h, r = i & (NH - 1), (r0 + NB * BR + (i >> 5) * PR) & (W - 1)
            return pltpu.make_async_copy(src.at[0, h, _rows(SK - W + r, PR, PR), :],
                                         dst.at[h, _rows((r - V0) & (W - 1), PR, PR), :], sem)
        return copy

    def short_ffn(j):
        src, dst = ((wg_h, wg_v), (wu_h, wu_v), (wd_h, wd_v))[j]

        def copy(i):
            rows = _rows((i & 1) * (F // 2) + (i >> 1) * OP, OP, OP)
            return pltpu.make_async_copy(src.at[rows, :], dst.at[rows, :], sem_w.at[1])
        return copy

    def short_wo(i):
        r, sem = wo_block((i >> 3) - NS)
        rest = i < NS * OB // OP
        return long_wo(jnp.where(rest, i & (NS - 1), NS - 1), 1,
                       jnp.where(rest, (RL + OB + (i >> 3) * OP) & (SR - 1), r + (i & 7) * OP), OP, sem)

    cargo = ((0, S_F, short_kv(k_h, k_v, K0, sem_k.at[1])), (S_F, S_V, None),
             (S_V, S_O, short_kv(v_h, v_v, V0, sem_v.at[VE])), (S_O, S_END, short_wo))

    def wait_all(ref, sem):
        pltpu.make_async_copy(ref, ref, sem).wait()

    started = [0]

    def run(n, k, t, work=None, carry=0):
        lo = started[0]
        hi = started[0] = lo + n * k
        for a, b, copy in cargo:
            if a < hi and b > lo:
                def body(i, c):
                    if S_K0 <= lo < S_K1:
                        n0 = k_due(lo + i * k)
                        pl.when(k_due(lo + (i + 1) * k) > n0)(lambda: start_k(n0))
                    for j in range(k):
                        if copy is None:
                            short_ffn(j)((lo - a) // 3 + i).start(priority=SHORT)
                        else:
                            copy(lo - a + i * k + j).start(priority=SHORT)
                        if work is None or j + 1 < k:
                            pl.delay(t)
                    return c if work is None else work(i, c)
                assert (max(a, lo) - lo) % k == 0 and (copy or (k == 3 and (lo - a) % 3 == 0))
                carry = jax.lax.fori_loop((max(a, lo) - lo) // k, (min(b, hi) - lo) // k, body, carry)
        return carry

    def idle_until(s):
        assert s >= started[0]
        if s > started[0]:
            run(s - started[0], 1, T_IDLE)

    assert k_due(S_K1) == NB * NH // KH and 3 * KRATE <= 1 << 16
    for n in range(2 * D // NS // OP):
        long_wq(n).start(priority=LONG)
    copy_x = pltpu.make_async_copy(x_h, x_v, sem_x.at[0])
    copy_wr = pltpu.make_async_copy(wr_h, wr_v, sem_x.at[1])
    copy_x.start(priority=SHORT)
    copy_wr.start(priority=SHORT)
    run(BURST, 1, T_BURST)

    q_v[...] = jnp.zeros(q_v.shape, F32)
    o_v[...] = jnp.zeros(o_v.shape, F32)
    idle_until(S_K0)
    idle_until(S_Q)
    copy_x.wait()
    copy_wr.wait()
    x = x_v[0].astype(F32)
    mean = jnp.mean(x, axis=-1, keepdims=True)
    var = jnp.mean(jnp.square(x - mean), axis=-1, keepdims=True)
    xn_b = ((x - mean) / jnp.sqrt(var + 1e-5)).astype(BF16)
    xn = xn_b.astype(F32)
    xn8 = jnp.broadcast_to(xn_b, (8, D))
    row = jax.lax.broadcasted_iota(jnp.int32, (8, DH), 0)

    def q_proj(i, c):
        w = wq_v[:, :, _rows(i * 2 * DH, 2 * DH, 2 * DH)].reshape(D, 2 * DH)
        q = jnp.dot(xn8, w, preferred_element_type=F32)
        g, j = i >> 2, (i & 3) * 2
        q_v[g] = jnp.where(row == j, q[:, :DH], jnp.where(row == j + 1, q[:, DH:], q_v[g]))
        return c
    wait_all(wq_v, sem_w.at[0])
    run(NH // 2, 3, T_QK, q_proj)
    idle_until(S_F)
    run((S_QK - S_F) // 3, 3, T_IDLE)

    def per_head(g, f):
        r = f(g * 8)
        for j in range(1, 8):
            r = jnp.where(row == j, f(g * 8 + j), r)
        return r

    k0, k1 = K0 - V0, K0 - V0 + KB * BR
    assert k_due(started[0]) >= KB * NH // KH and started[0] + 3 * KI >= S_K1 >= S_F
    assert 0 <= k0 <= DH and (KI // NG + 1) * DH <= k1

    def scores(i, c):
        g, t = i & (NG - 1), ((i >> 2) + 1) & (NT - 1)

        @pl.when(i == KI)
        def _():
            wait_all(k_v.at[:, pl.ds(k1, W - k1), :], sem_k.at[1])
            if k0:
                wait_all(k_v.at[:, pl.ds(0, k0), :], sem_k.at[1])
        q = q_v[g].astype(BF16)
        s_v[g, t] = per_head(g, lambda h: jax.lax.dot_general(
            q, k_v[h, _rows(t * DH, DH, DH), :], _NT, preferred_element_type=F32)) * (DH ** -0.5)
        return c
    wait_all(k_v.at[:, pl.ds(k0, k1 - k0), :], sem_k.at[0])
    n1 = (S_K1 - S_QK) // 3
    run(n1, 3, T_QK, scores)
    assert started[0] == S_K1

    @pl.loop(0, NB)
    def _(b):
        long_kv(v_h, v_v, slice(None), V0 + b * BR, BR, sem_v.at[jnp.where(b >= VE, b + 1, b)]).start(priority=LONG)

    run(NG * NT - n1, 3, T_QK, lambda i, c: scores(i + n1, c))

    def softmax(g, c):
        s = s_v[g]
        p = jnp.exp(s - jnp.max(jnp.max(s, axis=0), axis=-1, keepdims=True))
        s_v[g] = p
        l_v[g] = jnp.broadcast_to(jnp.sum(jnp.sum(p, axis=0), axis=-1, keepdims=True), (8, DH))
        return c
    run(NG, 3, T_O, softmax)

    def ffn(i, y):
        rows = _rows(jnp.minimum(i * DH, F - DH), DH, 32)
        new = jax.lax.broadcasted_iota(jnp.int32, (8, DH), 1) >= (i + 1) * DH - F
        gt = jax.lax.dot_general(xn8, wg_v[rows, :], _NT, preferred_element_type=F32)
        up = jax.lax.dot_general(xn8, wu_v[rows, :], _NT, preferred_element_type=F32)
        hid = jnp.where(new, jax.nn.silu(gt) * up, 0.0).astype(BF16)
        return y + jnp.dot(hid, wd_v[rows, :], preferred_element_type=F32)

    assert started[0] >= S_V + LAND
    for ref in (wg_v, wu_v, wd_v):
        wait_all(ref, sem_w.at[1])
    y = run(pl.cdiv(F, DH), 4, T_O, ffn, jnp.zeros((8, D), F32))
    r = jnp.sum(xn * wr_v[...].reshape(1, D).astype(F32), axis=-1, keepdims=True)
    gate = jax.nn.silu(xn + (xn * 0.0 + y * jax.nn.sigmoid(r)))

    idle_until(S_PV)

    @pl.loop(0, NOB - 1)
    def _(q):
        r0, sem = wo_block(q)
        long_wo(0, NS - 1, r0, OB, sem).start(priority=LONG)

    @pl.loop(0, NS - 2)
    def _(z):
        long_wo(z, 1, RL, OB, 3 + z).start(priority=LONG)

    last = [(RL + sum(LAST[:i]), nr, 1 + NS if i == 0 else 2 + NS + i) for i, nr in enumerate(LAST)]
    for piece in last:
        long_wo(NS - 2, 1, *piece).start(priority=LONG)

    assert S_PV + 3 * NG * VE >= S_O + LAND

    def values(i, c):
        g, u = i & (NG - 1), i >> 2
        b = jnp.where(u == VE, NB, u - (u > VE).astype(jnp.int32))
        pl.when(g == 0)(lambda: wait_all(v_v.at[:, _rows(b * BR, BR, BR), :], sem_v.at[u]))
        p = jnp.concatenate([s_v[g, 2 * b], s_v[g, 2 * b + 1]], axis=1).astype(BF16)
        o_v[g] += per_head(g, lambda h: jnp.dot(p, v_v[h, _rows(b * BR, BR, BR), :], preferred_element_type=F32))
        return c
    run(NG * (NB + 1), 3, T_PV, values)

    def normalize(g, c):
        o = o_v[g] / l_v[g]
        o_v[g] = o
        o = o.astype(BF16).astype(F32)
        for z in range(2):
            c_v[2 * g + z] = jnp.broadcast_to(o[4 * z + 3:4 * z + 4], (DH, DH)).T
        return c
    run(NG, 3, T_O, normalize)

    def head(acc, z, a):
        t = jnp.dot(o_v[z >> 1].astype(BF16), wo_v[z, pl.ds(a * DH, DH), :], preferred_element_type=F32)
        return acc + jnp.where(jax.lax.broadcasted_iota(jnp.int32, (8, D), 0) == (z & 1) * 4 + a, t, 0.0)

    def last_head(acc, z, r0, nr):
        coef = jnp.concatenate([c_v[z, pl.ds(r0 - 3 * DH, nr), :]] * (D // DH), axis=1)
        return acc + (wo_v[z, pl.ds(r0, nr), :].astype(F32) * coef).reshape(nr // 8, 8, D).sum(axis=0)

    def first(g, acc):
        for z in (2 * g, 2 * g + 1):
            acc = head(last_head(last_head(acc, z, 3 * DH, RL - 3 * DH), z, RL + OB, SR - RL - OB), z, 0)
        return acc

    def tail(z, acc):
        long_wo(z, 1, RL, OB, 3 + z).wait()
        return last_head(acc, z, RL, OB)

    idle_until(S_END - 18)
    for r0, r1 in ((0, O0 + 2 * OB), (RL - OB, RL), (RL + OB, SR)):
        wait_all(wo_v.at[:, pl.ds(r0, r1 - r0), :], sem_o.at[0])
    acc = run(NG, 2, T_O, first, jnp.zeros((8, D), F32))
    idle_until(S_END - 8)
    wait_all(wo_v.at[:, pl.ds(O0 + 2 * OB, 2 * OB), :], sem_o.at[1])
    acc = run(NG, 2, T_O, lambda g, acc: head(head(acc, 2 * g, 1), 2 * g + 1, 1), acc)
    wait_all(wo_v.at[:, pl.ds(O0 + 4 * OB, OB), :], sem_o.at[2])
    for z in range(NS):
        acc = head(acc, z, 2)
    acc = tail(NS - 1, jax.lax.fori_loop(0, NS - 2, tail, acc))
    for r0, nr, sem in last:
        long_wo(NS - 2, 1, r0, nr, sem).wait()
        acc = last_head(acc, NS - 2, r0, nr)

    s_out = jnp.broadcast_to(jnp.sum(acc, axis=0, keepdims=True), (8, D))
    out_ref[0] = (jnp.broadcast_to(x, (8, D)) + s_out * gate).astype(out_ref.dtype)[0:1]


@jax.jit
def pallas_recurrent_scan__sliding_block_cached__moe_arch_mod__decode_kernel(
    A_x: jax.Array,
    A_k_cache: jax.Array,
    A_v_cache: jax.Array,
    A_wq: jax.Array,
    A_wo: jax.Array,
    B_x: jax.Array,
    B_w_r: jax.Array,
    B_w_gate: jax.Array,
    B_w_up: jax.Array,
    B_w_down: jax.Array,
):
    del B_x
    hbm = pl.BlockSpec(memory_space=pltpu.HBM)
    dma = pltpu.SemaphoreType.DMA
    return pl.pallas_call(
        _kernel,
        out_shape=jax.ShapeDtypeStruct((1, 1, D), BF16),
        in_specs=[hbm] * 9,
        out_specs=pl.BlockSpec(memory_space=pltpu.VMEM),
        scratch_shapes=[
            pltpu.VMEM((1, 1, D), BF16),
            pltpu.VMEM((D,), BF16),
            pltpu.VMEM((NS, D // NS, NH * DH), BF16),
            pltpu.VMEM((NH, W, DH), BF16),
            pltpu.VMEM((NH, W, DH), BF16),
            pltpu.VMEM((NS, SR, D), BF16),
            pltpu.VMEM((F, D), BF16),
            pltpu.VMEM((F, D), BF16),
            pltpu.VMEM((F, D), BF16),
            pltpu.VMEM((NG, 8, DH), F32),
            pltpu.VMEM((NG, NT, 8, DH), F32),
            pltpu.VMEM((NG, 8, DH), F32),
            pltpu.VMEM((NG, 8, DH), F32),
            pltpu.VMEM((NS, DH, DH), F32),
            dma((2,)), dma((2,)), dma((2,)), dma((NB + 1,)), dma((2 + NS + len(LAST),)),
        ],
        compiler_params=pltpu.CompilerParams(
            vmem_limit_bytes=100 * 1024 * 1024,
            disable_semaphore_checks=True,
            disable_bounds_checks=True,
        ),
    )(A_x, A_k_cache, A_v_cache, A_wq.reshape(NS, D // NS, NH * DH), A_wo.reshape(NS, SR, D),
      B_w_r, B_w_gate.T, B_w_up.T, B_w_down)
```

```python
import jax
import jax.numpy as jnp
import jax.experimental.pallas as pl
import jax.experimental.pallas.tpu as pltpu

D = 512
NH = 32
DH = 128
SK = 32768
W = min(4096, max(256, SK // 4))
F = 1376
NG = NH // 8
NT = W // DH

BR, PR = 256, 32
NB = W // BR - 1
K0, V0 = 128, 64
K1 = 192
KH = 4
NS, SR = 8, 512
OB, OP = 64, 8
NOB = SR // OB - 1
O0 = 32
RL = O0 + (NOB - 1) * OB
O_CUTS = (0, O0 + 2 * OB, O0 + 4 * OB, RL - OB, RL, RL + OB, SR)
LAST = (32, 16, 16)

S_F = NH * BR // PR
S_V = S_F + 3 * F // OP
S_O = S_V + NH * BR // PR
S_END = S_O + (NS + NOB) * OB // OP
LAND = 8
S_K0, S_K1 = 56, 571
S_Q, S_QK, S_PV = 96, 388, 926
KB, KI = 9, 68
VE = 11
BURST, T_BURST = 16, 40
T_IDLE, T_QK, T_PV, T_O = 86, 36, 33, 20

BF16 = jnp.bfloat16
F32 = jnp.float32
_NT = (((1,), (1,)), ((), ()))
KRATE = pl.cdiv((NB * NH // KH) << 16, S_K1 - S_K0)
LONG, SHORT = 1, 0


def _rows(start, size, multiple):
    return pl.ds(start if isinstance(start, int) else pl.multiple_of(start, multiple), size)


def _kernel(x_h, k_h, v_h, wq_h, wo_h, wr_h, wg_h, wu_h, wd_h, out_ref,
            x_v, wr_v, wq_v, k_v, v_v, wo_v, wg_v, wu_v, wd_v, q_v, s_v, l_v, o_v, c_v,
            sem_x, sem_w, sem_k, sem_v, sem_o):
    def long_kv(src, dst, heads, r, nr, sem):
        return pltpu.make_async_copy(src.at[0, heads, _rows(SK - W + r, nr, PR), :],
                                     dst.at[heads, _rows(r - V0, nr, PR), :], sem)

    def start_k(n):
        b, h = (n * KH) >> 5, (n * KH) & (NH - 1)
        sem = sem_k.at[jnp.where(b >= KB, 1, 0)]
        long_kv(k_h, k_v, pl.ds(h, KH), K1 + b * BR, BR + K0 - K1, sem).start(priority=LONG)
        long_kv(k_h, k_v, pl.ds(h ^ (NH // 2), KH), K0 + b * BR, K1 - K0, sem).start(priority=LONG)

    def k_due(s):
        return ((s - S_K0) * KRATE) >> 16

    def copy_wo(z, nz, r, nr, i):
        idx = (pl.ds(z, nz), _rows(r, nr, OP), slice(None))
        return pltpu.make_async_copy(wo_h.at[idx], wo_v.at[idx], sem_o.at[i])

    def wo_block(q):
        return O0 + jnp.where(q == 0, 5, jnp.where(q == 6, 6, q - 1)) * OB

    def wo_sem(r):
        return sum((r >= cut).astype(jnp.int32) for cut in O_CUTS[1:-1])

    def long_wq(n):
        idx = (slice(None), _rows((n >> 1) * OP, OP, OP), _rows((n & 1) * (NH * DH // 2), NH * DH // 2, DH))
        return pltpu.make_async_copy(wq_h.at[idx], wq_v.at[idx], sem_w.at[0])

    def short_kv(src, dst, r0, sem):
        def copy(i):
            h, r = i & (NH - 1), (r0 + NB * BR + (i >> 5) * PR) & (W - 1)
            to = (r - V0) & (W - 1)
            return pltpu.make_async_copy(src.at[0, h, _rows(SK - W + r, PR, PR), :],
                                         dst.at[h, _rows(to, PR, PR), :], sem(to))
        return copy

    def short_ffn(j):
        src, dst = ((wg_h, wg_v), (wu_h, wu_v), (wd_h, wd_v))[j]

        def copy(i):
            rows = _rows((i & 1) * (F // 2) + (i >> 1) * OP, OP, OP)
            return pltpu.make_async_copy(src.at[rows, :], dst.at[rows, :], sem_w.at[1 + j])
        return copy

    def short_wo(i):
        rest = i < NS * OB // OP
        r = jnp.where(rest, (RL + OB + (i >> 3) * OP) & (SR - 1), wo_block((i >> 3) - NS) + (i & 7) * OP)
        return copy_wo(jnp.where(rest, i & (NS - 1), NS - 1), 1, r, OP, wo_sem(r))

    cargo = ((0, S_F, short_kv(k_h, k_v, K0, lambda to: sem_k.at[jnp.where(to < K0 - V0, 2, 1)])),
             (S_F, S_V, None),
             (S_V, S_O, short_kv(v_h, v_v, V0, lambda to: sem_v.at[VE])),
             (S_O, S_END, short_wo))

    def wait_all(ref, sem):
        pltpu.make_async_copy(ref, ref, sem).wait()

    started = [0]

    def run(n, k, t, work=None, carry=0):
        lo = started[0]
        hi = started[0] = lo + n * k
        for a, b, copy in cargo:
            if a < hi and b > lo:
                def body(i, c):
                    if S_K0 <= lo < S_K1:
                        n0 = k_due(lo + i * k)
                        pl.when(k_due(lo + (i + 1) * k) > n0)(lambda: start_k(n0))
                    for j in range(k):
                        if copy is None:
                            short_ffn(j)((lo - a) // 3 + i).start(priority=SHORT)
                        else:
                            copy(lo - a + i * k + j).start(priority=SHORT)
                        if work is None or j + 1 < k:
                            pl.delay(t)
                    return c if work is None else work(i, c)
                assert (max(a, lo) - lo) % k == 0 and (copy or (k == 3 and (lo - a) % 3 == 0))
                carry = jax.lax.fori_loop((max(a, lo) - lo) // k, (min(b, hi) - lo) // k, body, carry)
        return carry

    def idle_until(s):
        assert s >= started[0]
        if s > started[0]:
            run(s - started[0], 1, T_IDLE)

    assert k_due(S_K1) == NB * NH // KH and 3 * KRATE <= 1 << 16
    for n in range(2 * D // NS // OP):
        long_wq(n).start(priority=LONG)
    copy_x = pltpu.make_async_copy(x_h, x_v, sem_x.at[0])
    copy_wr = pltpu.make_async_copy(wr_h, wr_v, sem_x.at[1])
    copy_x.start(priority=SHORT)
    copy_wr.start(priority=SHORT)
    run(BURST, 1, T_BURST)

    q_v[...] = jnp.zeros(q_v.shape, F32)
    o_v[...] = jnp.zeros(o_v.shape, F32)
    idle_until(S_K0)
    idle_until(S_Q)
    copy_x.wait()
    copy_wr.wait()
    x = x_v[0].astype(F32)
    mean = jnp.mean(x, axis=-1, keepdims=True)
    var = jnp.mean(jnp.square(x - mean), axis=-1, keepdims=True)
    xn_b = ((x - mean) / jnp.sqrt(var + 1e-5)).astype(BF16)
    xn = xn_b.astype(F32)
    xn8 = jnp.broadcast_to(xn_b, (8, D))
    row = jax.lax.broadcasted_iota(jnp.int32, (8, DH), 0)

    def q_proj(i, c):
        w = wq_v[:, :, _rows(i * 2 * DH, 2 * DH, 2 * DH)].reshape(D, 2 * DH)
        q = jnp.dot(xn8, w, preferred_element_type=F32)
        g, j = i >> 2, (i & 3) * 2
        q_v[g] = jnp.where(row == j, q[:, :DH], jnp.where(row == j + 1, q[:, DH:], q_v[g]))
        return c
    wait_all(wq_v, sem_w.at[0])
    run(NH // 2, 3, T_O, q_proj)
    idle_until(S_F)
    run((S_QK - S_F) // 3, 3, T_IDLE)

    def per_head(g, f):
        r = f(g * 8)
        for j in range(1, 8):
            r = jnp.where(row == j, f(g * 8 + j), r)
        return r

    k0, k1 = K0 - V0, K0 - V0 + KB * BR
    assert k_due(started[0]) >= KB * NH // KH and started[0] + 3 * KI >= S_K1 >= S_F
    assert 0 < k0 <= DH and (KI // NG + 1) * DH <= k1

    def scores(i, c):
        g, t = i & (NG - 1), ((i >> 2) + 1) & (NT - 1)

        @pl.when(i == KI)
        def _():
            wait_all(k_v.at[:, pl.ds(k1, W - k1), :], sem_k.at[1])
            wait_all(k_v.at[:, pl.ds(0, k0), :], sem_k.at[2])
        q = q_v[g].astype(BF16)
        s_v[g, t] = per_head(g, lambda h: jax.lax.dot_general(
            q, k_v[h, _rows(t * DH, DH, DH), :], _NT, preferred_element_type=F32)) * (DH ** -0.5)
        return c
    wait_all(k_v.at[:, pl.ds(k0, k1 - k0), :], sem_k.at[0])
    n1 = (S_K1 - S_QK) // 3
    run(n1, 3, T_QK, scores)
    assert started[0] == S_K1

    @pl.loop(0, NB)
    def _(b):
        long_kv(v_h, v_v, slice(None), V0 + b * BR, BR, sem_v.at[jnp.where(b >= VE, b + 1, b)]).start(priority=LONG)

    run(NG * NT - n1, 3, T_QK, lambda i, c: scores(i + n1, c))

    def softmax(g, c):
        s = s_v[g]
        p = jnp.exp(s - jnp.max(jnp.max(s, axis=0), axis=-1, keepdims=True))
        s_v[g] = p
        l_v[g] = jnp.broadcast_to(jnp.sum(jnp.sum(p, axis=0), axis=-1, keepdims=True), (8, DH))
        return c
    run(NG, 3, T_O, softmax)

    def ffn(i, y):
        rows = _rows(jnp.minimum(i * DH, F - DH), DH, 32)
        new = jax.lax.broadcasted_iota(jnp.int32, (8, DH), 1) >= (i + 1) * DH - F
        gt = jax.lax.dot_general(xn8, wg_v[rows, :], _NT, preferred_element_type=F32)
        up = jax.lax.dot_general(xn8, wu_v[rows, :], _NT, preferred_element_type=F32)
        hid = jnp.where(new, jax.nn.silu(gt) * up, 0.0).astype(BF16)
        return y + jnp.dot(hid, wd_v[rows, :], preferred_element_type=F32)

    assert started[0] >= S_V + LAND
    for j, ref in enumerate((wg_v, wu_v, wd_v)):
        wait_all(ref, sem_w.at[1 + j])
    y = run(pl.cdiv(F, DH), 4, T_O, ffn, jnp.zeros((8, D), F32))
    r = jnp.sum(xn * wr_v[...].reshape(1, D).astype(F32), axis=-1, keepdims=True)
    gate = jax.nn.silu(xn + (xn * 0.0 + y * jax.nn.sigmoid(r)))

    idle_until(S_PV)

    @pl.loop(0, NOB - 1)
    def _(q):
        r0 = wo_block(q)
        copy_wo(0, NS - 1, r0, OB, wo_sem(r0)).start(priority=LONG)

    @pl.loop(0, NS - 2)
    def _(z):
        copy_wo(z, 1, RL, OB, 6 + z).start(priority=LONG)

    last = [(RL + sum(LAST[:i]), nr, 4 + NS + i) for i, nr in enumerate(LAST)]
    for piece in last:
        copy_wo(NS - 2, 1, *piece).start(priority=LONG)

    assert S_PV + 3 * NG * VE >= S_O + LAND

    def values(i, c):
        g, u = i & (NG - 1), i >> 2
        b = jnp.where(u == VE, NB, u - (u > VE).astype(jnp.int32))
        pl.when(g == 0)(lambda: wait_all(v_v.at[:, _rows(b * BR, BR, BR), :], sem_v.at[u]))
        p = jnp.concatenate([s_v[g, 2 * b], s_v[g, 2 * b + 1]], axis=1).astype(BF16)
        o_v[g] += per_head(g, lambda h: jnp.dot(p, v_v[h, _rows(b * BR, BR, BR), :], preferred_element_type=F32))
        return c
    run(NG * (NB + 1), 3, T_PV, values)

    def normalize(g, c):
        o = o_v[g] / l_v[g]
        o_v[g] = o
        o = o.astype(BF16).astype(F32)
        for z in range(2):
            c_v[2 * g + z] = jnp.broadcast_to(o[4 * z + 3:4 * z + 4], (DH, DH)).T
        return c
    run(NG, 3, T_O, normalize)

    def head(acc, z, a):
        t = jnp.dot(o_v[z >> 1].astype(BF16), wo_v[z, pl.ds(a * DH, DH), :], preferred_element_type=F32)
        return acc + jnp.where(jax.lax.broadcasted_iota(jnp.int32, (8, D), 0) == (z & 1) * 4 + a, t, 0.0)

    def last_head(acc, z, r0, nr):
        coef = jnp.concatenate([c_v[z, pl.ds(r0 - 3 * DH, nr), :]] * (D // DH), axis=1)
        return acc + (wo_v[z, pl.ds(r0, nr), :].astype(F32) * coef).reshape(nr // 8, 8, D).sum(axis=0)

    def wait_wo(i):
        wait_all(wo_v.at[:, pl.ds(O_CUTS[i], O_CUTS[i + 1] - O_CUTS[i]), :], sem_o.at[i])

    def first(g, acc):
        for z in (2 * g, 2 * g + 1):
            acc = head(last_head(last_head(acc, z, 3 * DH, RL - 3 * DH), z, RL + OB, SR - RL - OB), z, 0)
        return acc

    def tail(z, acc):
        copy_wo(z, 1, RL, OB, 6 + z).wait()
        return last_head(acc, z, RL, OB)

    idle_until(S_END - 18)
    for i in (0, 3, 5):
        wait_wo(i)
    acc = run(NG, 2, T_O, first, jnp.zeros((8, D), F32))
    idle_until(S_END - 8)
    wait_wo(1)
    acc = run(NG, 2, T_O, lambda g, acc: head(head(acc, 2 * g, 1), 2 * g + 1, 1), acc)
    wait_wo(2)
    for z in range(NS):
        acc = head(acc, z, 2)
    acc = jax.lax.fori_loop(0, NS - 2, tail, acc)
    wait_all(wo_v.at[NS - 1, pl.ds(RL, OB), :], sem_o.at[4])
    acc = last_head(acc, NS - 1, RL, OB)
    for r0, nr, sem in last:
        copy_wo(NS - 2, 1, r0, nr, sem).wait()
        acc = last_head(acc, NS - 2, r0, nr)

    s_out = jnp.broadcast_to(jnp.sum(acc, axis=0, keepdims=True), (8, D))
    out_ref[0] = (jnp.broadcast_to(x, (8, D)) + s_out * gate).astype(out_ref.dtype)[0:1]


@jax.jit
def pallas_recurrent_scan__sliding_block_cached__moe_arch_mod__decode_kernel(
    A_x: jax.Array,
    A_k_cache: jax.Array,
    A_v_cache: jax.Array,
    A_wq: jax.Array,
    A_wo: jax.Array,
    B_x: jax.Array,
    B_w_r: jax.Array,
    B_w_gate: jax.Array,
    B_w_up: jax.Array,
    B_w_down: jax.Array,
):
    del B_x
    hbm = pl.BlockSpec(memory_space=pltpu.HBM)
    dma = pltpu.SemaphoreType.DMA
    return pl.pallas_call(
        _kernel,
        out_shape=jax.ShapeDtypeStruct((1, 1, D), BF16),
        in_specs=[hbm] * 9,
        out_specs=pl.BlockSpec(memory_space=pltpu.VMEM),
        scratch_shapes=[
            pltpu.VMEM((1, 1, D), BF16),
            pltpu.VMEM((D,), BF16),
            pltpu.VMEM((NS, D // NS, NH * DH), BF16),
            pltpu.VMEM((NH, W, DH), BF16),
            pltpu.VMEM((NH, W, DH), BF16),
            pltpu.VMEM((NS, SR, D), BF16),
            pltpu.VMEM((F, D), BF16),
            pltpu.VMEM((F, D), BF16),
            pltpu.VMEM((F, D), BF16),
            pltpu.VMEM((NG, 8, DH), F32),
            pltpu.VMEM((NG, NT, 8, DH), F32),
            pltpu.VMEM((NG, 8, DH), F32),
            pltpu.VMEM((NG, 8, DH), F32),
            pltpu.VMEM((NS, DH, DH), F32),
            dma((2,)), dma((4,)), dma((3,)), dma((NB + 1,)), dma((4 + NS + len(LAST),)),
        ],
        compiler_params=pltpu.CompilerParams(
            vmem_limit_bytes=100 * 1024 * 1024,
            disable_semaphore_checks=True,
        ),
    )(A_x, A_k_cache, A_v_cache, A_wq.reshape(NS, D // NS, NH * DH), A_wo.reshape(NS, SR, D),
      B_w_r, B_w_gate.T, B_w_up.T, B_w_down)
```
